```python
import jax
import jax.numpy as jnp

def _softmax(x, axis=-1):
    return jax.nn.softmax(x, axis=axis)
def _gelu(x):
    return jax.nn.gelu(x, approximate=True)
def _silu(x):
    return jax.nn.silu(x)
def _sigmoid(x):
    return jax.nn.sigmoid(x)
def _layernorm(x, axis=-1, eps=1e-5):
    m = jnp.mean(x, axis=axis, keepdims=True)
    v = jnp.var(x, axis=axis, keepdims=True)
    return (x - m) / jnp.sqrt(v + eps)
def _scatter_add(tgt, idx, src, axis=0):
    return tgt.at[idx].add(src)
def _segment_sum(src, seg, n):
    return jax.ops.segment_sum(src, seg, n)
class _Rng:
    def __init__(self, key):
        self._k = key
    def _next(self):
        self._k, sub = jax.random.split(self._k)
        return sub
    def normal(self, shape):
        return jax.random.normal(self._next(), shape, dtype=jnp.bfloat16)
    def randint(self, lo, hi, shape):
        return jax.random.randint(self._next(), shape, lo, hi, dtype=jnp.int32)
    def uniform(self, shape, lo=0.0, hi=1.0):
        return jax.random.uniform(self._next(), shape, jnp.bfloat16, lo, hi)
    def permutation(self, n):
        return jax.random.permutation(self._next(), n)


kernel_name = 'standalone__gqa_softmax__near_ridge'

def setup_inputs():
    _rng = _Rng(jax.random.key(int.from_bytes(__import__("os").urandom(4), "little")))
    _w = (lambda a: (lambda t: t.astype(jnp.bfloat16) if jnp.issubdtype(t.dtype, jnp.floating) else t)(jnp.asarray(a)))
    B, Hq, Hkv, Sq, Sk, D = 16, 32, 32, 848, 512, 192
    return {
        "q": _w((lambda *s: _rng.normal(s) * 0.05)(B, Hq, Sq, D)),
        "k": _w((lambda *s: _rng.normal(s) * 0.05)(B, Hkv, Sk, D)),
        "v": _w((lambda *s: _rng.normal(s) * 0.05)(B, Hkv, Sk, D)),
    }

def reference(q, k, v):
    B, Hq, Sq, D = q.shape
    Hkv = k.shape[1]
    rep = Hq // Hkv
    k = jnp.repeat(k, rep, axis=1)
    v = jnp.repeat(v, rep, axis=1)
    scale = D ** -0.5
    scores = jnp.einsum("bhqd,bhkd->bhqk", q, k) * scale
    p = _softmax(scores, axis=-1)
    return jnp.einsum("bhqk,bhkd->bhqd", p, v)
```

```python
import functools
import math

import jax
import jax.numpy as jnp
import jax.experimental.pallas as pl
import jax.experimental.pallas.tpu as pltpu


def _attn_kernel(q_ref, k_ref, v_ref, o_ref, *, heads, c):
    for h in range(heads):
        qt = q_ref[h]
        kt = k_ref[h]
        vt = v_ref[h]
        st = jax.lax.dot_general(
            kt, qt, (((0,), (0,)), ((), ())), preferred_element_type=jnp.float32
        )
        m = jnp.max(st, axis=0, keepdims=True)
        p = jnp.exp2((st - m) * c)
        l = jnp.sum(p, axis=0, keepdims=True)
        ot = jnp.dot(vt, p.astype(vt.dtype), preferred_element_type=jnp.float32)
        o_ref[h] = (ot * (1.0 / l)).astype(o_ref.dtype)


@jax.jit
def pallas_standalone__gqa_softmax__near_ridge_kernel(
    q: jax.Array,
    k: jax.Array,
    v: jax.Array,
):
    B, Hq, Sq, D = q.shape
    Hkv, Sk = k.shape[1], k.shape[2]
    assert Hq == Hkv
    heads = 1
    n = B * Hq
    qt = jnp.swapaxes(q, 2, 3).reshape(n, D, Sq)
    kt = jnp.swapaxes(k, 2, 3).reshape(n, D, Sk)
    vt = jnp.swapaxes(v, 2, 3).reshape(n, D, Sk)
    c = (D ** -0.5) * math.log2(math.e)
    ot = pl.pallas_call(
        functools.partial(_attn_kernel, heads=heads, c=c),
        grid=(n // heads,),
        in_specs=[
            pl.BlockSpec((heads, D, Sq), lambda i: (i, 0, 0)),
            pl.BlockSpec((heads, D, Sk), lambda i: (i, 0, 0)),
            pl.BlockSpec((heads, D, Sk), lambda i: (i, 0, 0)),
        ],
        out_specs=pl.BlockSpec((heads, D, Sq), lambda i: (i, 0, 0)),
        out_shape=jax.ShapeDtypeStruct((n, D, Sq), q.dtype),
        compiler_params=pltpu.CompilerParams(
            dimension_semantics=("parallel",),
            vmem_limit_bytes=64 * 1024 * 1024,
        ),
    )(qt, kt, vt)
    return jnp.swapaxes(ot.reshape(B, Hq, D, Sq), 2, 3)
```

```python
import functools
import math

import jax
import jax.numpy as jnp
import jax.experimental.pallas as pl
import jax.experimental.pallas.tpu as pltpu

_F32 = jnp.float32
_BF16 = jnp.bfloat16


def _dot(a, b):
    return jnp.dot(a, b, preferred_element_type=_F32)


def _prep_k(k_ref, h):
    n = k_ref.shape[2] // 2

    def blk(r, col):
        return k_ref[h, 64 * r:64 * (r + 1), n * col:n * (col + 1)].astype(_F32)

    k1a, k1b, k1c = blk(0, 0), blk(1, 0), blk(2, 0)
    k2a, k2b, k2c = blk(0, 1), blk(1, 1), blk(2, 1)

    def cat(a, b):
        return jnp.concatenate([a, b], 0).astype(_BF16).T

    return cat(k1a, k2b), cat(k1b - k2b, k1c), cat(k2a - k1a, k2c)


def _attn_kernel(q_ref, k_ref, v_ref, o_ref, s_ref, *, heads, c, tiles, lag):
    sk = k_ref.shape[2]
    half = sk // 2
    items = [(h, a, b) for h in range(heads) for (a, b) in tiles]
    ks, vs, maxes, probs = {}, {}, {}, {}

    def qk(i):
        h, a, b = items[i]
        w = b - a
        if h not in ks:
            ks[h] = _prep_k(k_ref, h)
        l1, l2, l3 = ks[h]
        w1 = q_ref[h, 0:2, :, a:b].reshape(128, w)
        w2 = q_ref[h, 1:3, :, a:b].reshape(128, w)
        w3 = jnp.concatenate(
            [q_ref[h, 0:1, :, a:b], q_ref[h, 2:3, :, a:b]], 0).reshape(128, w)
        t1 = _dot(l1, w1)
        s1 = t1 + _dot(l2, w2)
        s2 = t1 + _dot(l3, w3)
        maxes[i] = jnp.max(jnp.maximum(s1, s2), axis=0, keepdims=True)
        slot = i % s_ref.shape[0]
        s_ref[slot, 0:half, 0:w] = s1
        s_ref[slot, half:sk, 0:w] = s2

    def softmax(i):
        h, a, b = items[i]
        w = b - a
        m = jnp.broadcast_to(maxes.pop(i), (16, w))
        acc, es = None, []
        for r in range(0, sk, 16):
            e = jnp.exp2((s_ref[i % s_ref.shape[0], r:r + 16, 0:w] - m) * c)
            part = e[0:8] + e[8:16]
            acc = part if acc is None else acc + part
            es.append(e)
        l = jnp.sum(acc, axis=0, keepdims=True)
        probs[i] = (jnp.concatenate(es, 0).astype(_BF16), 1.0 / l)

    def pv(i):
        h, a, b = items[i]
        if h not in vs:
            vs[h] = v_ref[h]
        p, r = probs.pop(i)
        o_ref[h, :, a:b] = (_dot(vs[h], p) * r).astype(o_ref.dtype)

    n = len(items)
    for s in range(n + lag):
        if s < n:
            qk(s)
        if 0 <= s - 1 < n:
            softmax(s - 1)
        if 0 <= s - lag < n:
            pv(s - lag)


@jax.jit
def pallas_standalone__gqa_softmax__near_ridge_kernel(
    q: jax.Array,
    k: jax.Array,
    v: jax.Array,
):
    B, Hq, Sq, D = q.shape
    Hkv, Sk = k.shape[1], k.shape[2]
    assert Hq == Hkv and D == 192
    heads, lag = 8, 3
    n = B * Hq
    qt = jnp.swapaxes(q, 2, 3).reshape(n, 3, D // 3, Sq)
    kt = jnp.swapaxes(k, 2, 3).reshape(n, D, Sk)
    vt = jnp.swapaxes(v, 2, 3).reshape(n, D, Sk)
    c = (D ** -0.5) * math.log2(math.e)
    tiles = [(a, min(a + 128, Sq)) for a in range(0, Sq, 128)]
    ot = pl.pallas_call(
        functools.partial(_attn_kernel, heads=heads, c=c, tiles=tiles, lag=lag),
        grid=(n // heads,),
        in_specs=[
            pl.BlockSpec((heads, 3, D // 3, Sq), lambda i: (i, 0, 0, 0)),
            pl.BlockSpec((heads, D, Sk), lambda i: (i, 0, 0)),
            pl.BlockSpec((heads, D, Sk), lambda i: (i, 0, 0)),
        ],
        out_specs=pl.BlockSpec((heads, D, Sq), lambda i: (i, 0, 0)),
        out_shape=jax.ShapeDtypeStruct((n, D, Sq), q.dtype),
        scratch_shapes=[pltpu.VMEM((lag + 1, Sk, 128), _F32)],
        compiler_params=pltpu.CompilerParams(
            dimension_semantics=("parallel",),
            vmem_limit_bytes=64 * 1024 * 1024,
            flags={"XLA_TPU_FORCE_LP_LLO_SCHEDULER": True},
        ),
    )(qt, kt, vt)
    return jnp.swapaxes(ot.reshape(B, Hq, D, Sq), 2, 3)
```

```python
import functools
import math

import jax
import jax.numpy as jnp
import jax.experimental.pallas as pl
import jax.experimental.pallas.tpu as pltpu

_F32 = jnp.float32
_BF16 = jnp.bfloat16
_U32 = jnp.uint32

_BIG = 8
_SMALL = 2
_N_FIRST = 10
_N_LAST = 2
_PV_LAG = 3
_REM_POS = 1
_K_PREP_POS = 4
_S_SLOTS = 4


def _dot(a, b):
    return jnp.dot(a, b, preferred_element_type=_F32)


def _dot_tn(a, b):
    return jax.lax.dot_general(a, b, (((0,), (0,)), ((), ())), preferred_element_type=_F32)


def _dot_nt(a, b):
    return jax.lax.dot_general(a, b, (((1,), (1,)), ((), ())), preferred_element_type=_F32)


def _sum(xs):
    return functools.reduce(lambda a, b: a + b, xs)


def _prep_k(k_ref):
    half = k_ref.shape[1] // 2

    def blk(r, col):
        return k_ref[64 * r:64 * (r + 1), half * col:half * (col + 1)].astype(_F32)

    k1a, k1b, k1c = blk(0, 0), blk(1, 0), blk(2, 0)
    k2a, k2b, k2c = blk(0, 1), blk(1, 1), blk(2, 1)

    def cat(a, b):
        return jnp.concatenate([a, b], 0).astype(_BF16)

    kn = (cat(k1a, k2b), cat(k1b - k2b, k1c), cat(k2a - k1a, k2c))
    return kn, tuple(x.T for x in kn)


def _save_k(k, kn_ref, kt_ref):
    for j in range(3):
        kn_ref[j] = pltpu.bitcast(k[0][j], _U32)
        kt_ref[j] = pltpu.bitcast(k[1][j], _U32)


def _load_k(kn_ref, kt_ref):
    return (tuple(pltpu.bitcast(kn_ref[j], _BF16) for j in range(3)),
            tuple(pltpu.bitcast(kt_ref[j], _BF16) for j in range(3)))


def _group(q_ref, k_ref, v_ref, o_ref, kn_ref, kt_ref, s_refs, zero, scale_log2e):
    heads, _, sq = o_ref.shape
    sk = k_ref.shape[2]
    tiles = [(a, a + 128) for a in range(0, sq - 127, 128)]
    if sq % 128:
        tiles.insert(_REM_POS, (sq - sq % 128, sq))
    items = [(h, a, b) for h in range(heads) for a, b in tiles]
    full = [i for i, (_, a, b) in enumerate(items) if b - a == 128]
    s_ref = {i: s_refs[j % len(s_refs)] for j, i in enumerate(full)}
    ks = {0: _load_k(kn_ref, kt_ref)}
    vs, scores, probs = {}, {}, {}

    def qk(i):
        h, a, b = items[i]
        w = b - a
        q_ab = q_ref[h, 0:2, :, a:b].reshape(128, w)
        q_bc = q_ref[h, 1:3, :, a:b].reshape(128, w)
        q_ac = jnp.concatenate(
            [q_ref[h, 0:1, :, a:b], q_ref[h, 2:3, :, a:b]], 0).reshape(128, w)
        if w == 128:
            k1, k2, k3 = ks[h][1]
            t1 = _dot(k1, q_ab)
            s1 = t1 + _dot(k2, q_bc)
            s2 = t1 + _dot(k3, q_ac)
            m = jnp.max(jnp.maximum(s1, s2), axis=0, keepdims=True)
            s_ref[i][0, 0:sk // 2, :] = s1
            s_ref[i][0, sk // 2:sk, :] = s2
            scores[i] = m
        else:
            k1, k2, k3 = ks[h][0]
            t1 = _dot_tn(q_ab, k1)
            s1 = t1 + _dot_tn(q_bc, k2)
            s2 = t1 + _dot_tn(q_ac, k3)
            m = jnp.max(jnp.maximum(s1, s2), axis=1, keepdims=True)
            scores[i] = (s1, s2, m)

    def softmax(i):
        _, a, b = items[i]
        w = b - a
        if w == 128:
            m = jnp.broadcast_to(scores.pop(i), (8, w))
            es = [jnp.exp2((s_ref[i][zero, r:r + 8, :] - m) * scale_log2e)
                  for r in range(0, sk, 8)]
            inv = 1.0 / jnp.sum(_sum(es), axis=0, keepdims=True)
            p = [jnp.concatenate(es[j:j + 16], 0).astype(_BF16) for j in range(0, sk // 8, 16)]
            probs[i] = (p, inv)
        else:
            s1, s2, m = scores.pop(i)
            m = jnp.broadcast_to(m, (w, 128))
            es = [jnp.exp2((s[:, j:j + 128] - m) * scale_log2e)
                  for s in (s1, s2) for j in range(0, sk // 2, 128)]
            inv = 1.0 / jnp.sum((es[0] + es[1]) + (es[2] + es[3]), axis=1, keepdims=True)
            probs[i] = [(e * inv).astype(_BF16) for e in es]

    def pv(i):
        h, a, b = items[i]
        if h not in vs:
            vs[h] = [(v_ref[h, 0:128, j:j + 128], v_ref[h, :, j:j + 128],
                      v_ref[h, 128:192, j:j + 128]) for j in range(0, sk, 128)]
        if b - a == 128:
            p, inv = probs.pop(i)
            o = _sum([_dot(v[1], pj) for v, pj in zip(vs[h], p)])
            o_ref[h, :, a:b] = (o * inv).astype(o_ref.dtype)
        else:
            p = probs.pop(i)
            o_lo = _sum([_dot_nt(pj, v[0]) for v, pj in zip(vs[h], p)])
            o_hi = _sum([_dot_nt(v[2], pj) for v, pj in zip(vs[h], p)])
            o_ref[h, 0:128, a:b] = o_lo.astype(o_ref.dtype).T
            o_ref[h, 128:192, a:b] = o_hi.astype(o_ref.dtype)

    n = len(items)
    for step in range(n + _PV_LAG):
        h, t = divmod(step, len(tiles))
        if step < n and t == _K_PREP_POS:
            ks[h + 1] = _prep_k(k_ref.at[h])
            if h + 1 == heads:
                _save_k(ks[heads], kn_ref, kt_ref)
        if step < n:
            qk(step)
        if 0 <= step - 1 < n:
            softmax(step - 1)
        if 0 <= step - _PV_LAG:
            pv(step - _PV_LAG)


def _attn_kernel(q_hbm, k_hbm, v_hbm, o_hbm,
                 qs, ks, vs, os, qb, kb, vb, ob, kn_ref, kt_ref,
                 sem_si, sem_so, sem_bi, sem_bo, *s_refs, scale_log2e):
    n_heads = q_hbm.shape[0]
    n_big = (n_heads - _SMALL * (_N_FIRST + _N_LAST)) // _BIG
    big0 = _SMALL * _N_FIRST
    last0 = big0 + _BIG * n_big
    assert last0 + _SMALL * _N_LAST == n_heads and n_big >= 2
    assert _N_FIRST >= _BIG and _N_FIRST % 2 == 0 and _N_LAST == 2
    copy = pltpu.make_async_copy

    def start_loads(head, n, dsts, sem):
        for src, dst, off in zip((k_hbm, q_hbm, v_hbm), dsts, (1, 0, 0)):
            copy(src.at[pl.ds(head + off, n)], dst, sem).start()

    def wait_loads(dsts, sem):
        for dst in dsts:
            copy(dst, dst, sem).wait()

    def small_in(slot):
        return (ks.at[slot], qs.at[slot], vs.at[slot]), sem_si.at[slot]

    def big_in(slot):
        return (kb.at[slot], qb.at[slot], vb.at[slot]), sem_bi.at[slot]

    def small_out(head, slot):
        return copy(os.at[slot], o_hbm.at[pl.ds(head, _SMALL)], sem_so.at[slot])

    def big_out(i):
        return copy(ob.at[i & 1], o_hbm.at[pl.ds(big0 + _BIG * i, _BIG)], sem_bo.at[i & 1])

    def run(bufs, slot, it):
        zero = jax.lax.shift_right_logical(it, 30)
        _group(*(x.at[slot] for x in bufs), kn_ref, kt_ref, s_refs, zero, scale_log2e)

    k0 = copy(k_hbm.at[0], kb.at[1, 0], sem_bi.at[1])
    k0.start()
    start_loads(0, _SMALL, *small_in(0))
    k0.wait()
    _save_k(_prep_k(kb.at[1, 0]), kn_ref, kt_ref)

    def first_step(j, _):
        slot = j & 1

        @pl.when(j + 1 < _N_FIRST)
        def _():
            start_loads(_SMALL * (j + 1), _SMALL, *small_in(1 - slot))

        @pl.when(j >= _N_FIRST - _BIG)
        def _():
            p = j - (_N_FIRST - _BIG)
            dsts = tuple(x.at[0, pl.ds(p, 1)] for x in (kb, qb, vb))
            start_loads(big0 + p, 1, dsts, sem_bi.at[0])

        wait_loads(*small_in(slot))

        @pl.when(j >= 2)
        def _():
            small_out(_SMALL * (j - 2), slot).wait()

        run((qs, ks, vs, os), slot, j)
        small_out(_SMALL * j, slot).start()

    jax.lax.fori_loop(0, _N_FIRST, first_step, None)

    start_loads(big0 + _BIG, _BIG, *big_in(1))
    start_loads(last0, _SMALL, *small_in(0))
    tail = n_heads - _SMALL
    copy(k_hbm.at[pl.ds(tail + 1, _SMALL - 1)], ks.at[1, pl.ds(0, _SMALL - 1)],
         sem_si.at[1]).start()
    copy(k_hbm.at[n_heads - 1], ks.at[1, _SMALL - 1], sem_si.at[1]).start()
    copy(q_hbm.at[pl.ds(tail, _SMALL)], qs.at[1], sem_si.at[1]).start()
    copy(v_hbm.at[pl.ds(tail, _SMALL)], vs.at[1], sem_si.at[1]).start()

    def big_step(i, _):
        slot = i & 1
        wait_loads(*big_in(slot))

        @pl.when(i >= 2)
        def _():
            big_out(i - 2).wait()

        run((qb, kb, vb, ob), slot, i)

        @pl.when(i + 2 < n_big)
        def _():
            start_loads(big0 + _BIG * (i + 2), _BIG, *big_in(slot))

        big_out(i).start()

    jax.lax.fori_loop(0, n_big, big_step, None)

    for j in range(_N_FIRST - 2, _N_FIRST):
        small_out(_SMALL * j, j & 1).wait()

    def last_step(j, _):
        wait_loads(*small_in(j))
        run((qs, ks, vs, os), j, j)
        small_out(last0 + _SMALL * j, j).start()

    jax.lax.fori_loop(0, _N_LAST, last_step, None)

    big_out(n_big - 2).wait()
    big_out(n_big - 1).wait()
    for j in range(_N_LAST):
        small_out(last0 + _SMALL * j, j).wait()


@jax.jit
def pallas_standalone__gqa_softmax__near_ridge_kernel(
    q: jax.Array,
    k: jax.Array,
    v: jax.Array,
):
    B, Hq, Sq, D = q.shape
    Hkv, Sk = k.shape[1], k.shape[2]
    assert Hq == Hkv and D == 192 and Sk == 512
    n = B * Hq
    qt = jnp.swapaxes(q, 2, 3).reshape(n, 3, D // 3, Sq)
    kt = jnp.swapaxes(k, 2, 3).reshape(n, D, Sk)
    vt = jnp.swapaxes(v, 2, 3).reshape(n, D, Sk)

    def buffers(heads):
        return [pltpu.VMEM((2, heads, 3, D // 3, Sq), q.dtype),
                pltpu.VMEM((2, heads, D, Sk), k.dtype),
                pltpu.VMEM((2, heads, D, Sk), v.dtype),
                pltpu.VMEM((2, heads, D, Sq), q.dtype)]

    ot = pl.pallas_call(
        functools.partial(_attn_kernel, scale_log2e=(D ** -0.5) * math.log2(math.e)),
        in_specs=[pl.BlockSpec(memory_space=pl.ANY)] * 3,
        out_specs=pl.BlockSpec(memory_space=pl.ANY),
        out_shape=jax.ShapeDtypeStruct((n, D, Sq), q.dtype),
        scratch_shapes=[
            *buffers(_SMALL),
            *buffers(_BIG),
            pltpu.VMEM((3, 64, Sk // 2), _U32),
            pltpu.VMEM((3, Sk // 4, 128), _U32),
            *[pltpu.SemaphoreType.DMA((2,))] * 4,
            *[pltpu.VMEM((1, Sk, 128), _F32)] * _S_SLOTS,
        ],
        compiler_params=pltpu.CompilerParams(
            vmem_limit_bytes=64 * 1024 * 1024,
            disable_bounds_checks=True,
            flags={"XLA_TPU_FORCE_LP_LLO_SCHEDULER": True},
        ),
    )(qt, kt, vt)
    return jnp.swapaxes(ot.reshape(B, Hq, D, Sq), 2, 3)
```

```python
import functools
import math

import jax
import jax.numpy as jnp
import jax.experimental.pallas as pl
import jax.experimental.pallas.tpu as pltpu

_F32 = jnp.float32
_BF16 = jnp.bfloat16
_U32 = jnp.uint32

_BIG = 12
_SMALL = 2
_N_FIRST = 13
_N_LAST = 3
_EARLY = 4
_PV_LAG = 3
_REM_POS = 3
_K_PREP_POS = 4
_S_SLOTS = 4


def _dot(a, b):
    return jnp.dot(a, b, preferred_element_type=_F32)


def _dot_tn(a, b):
    return jax.lax.dot_general(a, b, (((0,), (0,)), ((), ())), preferred_element_type=_F32)


def _dot_nt(a, b):
    return jax.lax.dot_general(a, b, (((1,), (1,)), ((), ())), preferred_element_type=_F32)


def _sum(xs):
    return functools.reduce(lambda a, b: a + b, xs)


def _reciprocal(x):
    r = pl.reciprocal(x, approx=True)
    return r * (2.0 - x * r)


def _prep_k(k_ref, scale_log2e):
    half = k_ref.shape[1] // 2

    def blk(r, col):
        x = k_ref[64 * r:64 * (r + 1), half * col:half * (col + 1)]
        return x.astype(_F32) * scale_log2e

    k1a, k1b, k1c = blk(0, 0), blk(1, 0), blk(2, 0)
    k2a, k2b, k2c = blk(0, 1), blk(1, 1), blk(2, 1)

    def cat(a, b):
        return jnp.concatenate([a, b], 0).astype(_BF16)

    kn = (cat(k1a, k2b), cat(k1b - k2b, k1c), cat(k2a - k1a, k2c))
    return kn, tuple(x.T for x in kn)


def _save_k(k, kn_ref, kt_ref):
    for j in range(3):
        kn_ref[j] = pltpu.bitcast(k[0][j], _U32)
        kt_ref[j] = pltpu.bitcast(k[1][j], _U32)


def _load_k(kn_ref, kt_ref):
    return (tuple(pltpu.bitcast(kn_ref[j], _BF16) for j in range(3)),
            tuple(pltpu.bitcast(kt_ref[j], _BF16) for j in range(3)))


def _group(q_ref, k_ref, v_ref, o_ref, kn_ref, kt_ref, s_refs, zero, scale_log2e):
    heads, _, sq = o_ref.shape
    sk = k_ref.shape[2]
    tiles = [(a, a + 128) for a in range(0, sq - 127, 128)]
    if sq % 128:
        tiles.insert(_REM_POS, (sq - sq % 128, sq))
    items = [(h, a, b) for h in range(heads) for a, b in tiles]
    full = [i for i, (_, a, b) in enumerate(items) if b - a == 128]
    s_ref = {i: s_refs[j % len(s_refs)] for j, i in enumerate(full)}
    ks = {0: _load_k(kn_ref, kt_ref)}
    vs, scores, probs = {}, {}, {}

    def qk(i):
        h, a, b = items[i]
        w = b - a
        q_ab = q_ref[h, 0:2, :, a:b].reshape(128, w)
        q_bc = q_ref[h, 1:3, :, a:b].reshape(128, w)
        q_ac = jnp.concatenate(
            [q_ref[h, 0:1, :, a:b], q_ref[h, 2:3, :, a:b]], 0).reshape(128, w)
        if w == 128:
            k1, k2, k3 = ks[h][1]
            t1 = _dot(k1, q_ab)
            s1 = t1 + _dot(k2, q_bc)
            s2 = t1 + _dot(k3, q_ac)
            scores[i] = jnp.max(jnp.maximum(s1, s2), axis=0, keepdims=True)
            s_ref[i][0, 0:sk // 2, :] = s1
            s_ref[i][0, sk // 2:sk, :] = s2
        else:
            k1, k2, k3 = ks[h][0]
            t1 = _dot_tn(q_ab, k1)
            s1 = t1 + _dot_tn(q_bc, k2)
            s2 = t1 + _dot_tn(q_ac, k3)
            scores[i] = (s1, s2, jnp.max(jnp.maximum(s1, s2), axis=1, keepdims=True))

    def softmax(i):
        _, a, b = items[i]
        w = b - a
        if w == 128:
            m = jnp.broadcast_to(scores.pop(i), (8, w))
            acc, es, p = None, [], []
            for r in range(0, sk, 8):
                e = jnp.exp2(s_ref[i][zero, r:r + 8, :] - m)
                acc = e if acc is None else acc + e
                es.append(e)
                if len(es) == 16:
                    p.append(jnp.concatenate(es, 0).astype(_BF16))
                    es = []
            probs[i] = (p, _reciprocal(jnp.sum(acc, axis=0, keepdims=True)))
        else:
            s1, s2, m = scores.pop(i)
            m = jnp.broadcast_to(m, (w, 128))
            es = [jnp.exp2(s[:, j:j + 128] - m)
                  for s in (s1, s2) for j in range(0, sk // 2, 128)]
            inv = _reciprocal(
                jnp.sum((es[0] + es[1]) + (es[2] + es[3]), axis=1, keepdims=True))
            probs[i] = ([e.astype(_BF16) for e in es], inv)

    def pv(i):
        h, a, b = items[i]
        if h not in vs:
            vs[h] = [(v_ref[h, 0:128, j:j + 128], v_ref[h, :, j:j + 128],
                      v_ref[h, 128:192, j:j + 128]) for j in range(0, sk, 128)]
        p, inv = probs.pop(i)
        if b - a == 128:
            o = _sum([_dot(v[1], pj) for v, pj in zip(vs[h], p)])
            o_ref[h, :, a:b] = (o * inv).astype(o_ref.dtype)
        else:
            o_lo = _sum([_dot_nt(pj, v[0]) for v, pj in zip(vs[h], p)])
            o_hi = _sum([_dot_nt(v[2], pj) for v, pj in zip(vs[h], p)])
            inv = jnp.broadcast_to(inv, (b - a, 128))
            o_lo = o_lo * inv
            o_hi = o_hi * inv.T[0:64]
            o_ref[h, 0:128, a:b] = o_lo.astype(o_ref.dtype).T
            o_ref[h, 128:192, a:b] = o_hi.astype(o_ref.dtype)

    n = len(items)
    for step in range(n + _PV_LAG):
        h, t = divmod(step, len(tiles))
        if step < n and t == _K_PREP_POS:
            ks[h + 1] = _prep_k(k_ref.at[h], scale_log2e)
            if h + 1 == heads:
                _save_k(ks[heads], kn_ref, kt_ref)
        if step < n:
            qk(step)
        if 0 <= step - 1 < n:
            softmax(step - 1)
        if 0 <= step - _PV_LAG:
            pv(step - _PV_LAG)


def _attn_kernel(q_hbm, k_hbm, v_hbm, o_hbm,
                 q_small, k_small, v_small, o_small, q_big, k_big, v_big, o_big,
                 kn_ref, kt_ref, sem_si, sem_so, sem_bi, sem_bo, *s_refs, scale_log2e):
    n_heads = q_hbm.shape[0]
    n_big = (n_heads - _SMALL * (_N_FIRST + _N_LAST)) // _BIG
    big0 = _SMALL * _N_FIRST
    last0 = big0 + _BIG * n_big
    assert last0 + _SMALL * _N_LAST == n_heads and n_big >= 2
    assert _N_FIRST >= max(_BIG, _N_LAST) and _N_LAST >= 2
    copy = pltpu.make_async_copy

    def small(ref, j):
        return ref.at[pl.ds(_SMALL * j, _SMALL)]

    def start_loads(head, n, dsts, sem):
        for src, dst, off in zip((k_hbm, q_hbm, v_hbm), dsts, (1, 0, 0)):
            copy(src.at[pl.ds(head + off, n)], dst, sem).start()

    def wait_loads(dsts, sem):
        for dst in dsts:
            copy(dst, dst, sem).wait()

    def small_in(j, sem):
        return tuple(small(x, j) for x in (k_small, q_small, v_small)), sem_si.at[sem]

    def big_in(slot):
        return tuple(x.at[slot] for x in (k_big, q_big, v_big)), sem_bi.at[slot]

    def big_out(i):
        return copy(o_big.at[i & 1], o_hbm.at[pl.ds(big0 + _BIG * i, _BIG)], sem_bo.at[i & 1])

    def last_out(j):
        return copy(small(o_small, _N_FIRST + j),
                    o_hbm.at[pl.ds(last0 + _SMALL * j, _SMALL)], sem_so.at[j])

    first_out = [
        copy(o_small.at[pl.ds(a, b - a)], o_hbm.at[pl.ds(a, b - a)], sem_so.at[_N_LAST + j])
        for j, (a, b) in enumerate(((0, _EARLY), (_EARLY, big0)))]

    def run(bufs, it):
        zero = jax.lax.shift_right_logical(it, 30)
        _group(*bufs, kn_ref, kt_ref, s_refs, zero, scale_log2e)

    k0 = copy(k_hbm.at[0], k_big.at[1, 0], sem_bi.at[1])
    k0.start()
    start_loads(0, _SMALL, *small_in(0, 0))
    k0.wait()
    _save_k(_prep_k(k_big.at[1, 0], scale_log2e), kn_ref, kt_ref)

    def first_step(j, _):
        wait_loads(*small_in(j, j & 1))

        @pl.when(j + 1 < _N_FIRST)
        def _():
            start_loads(_SMALL * (j + 1), _SMALL, *small_in(j + 1, (j + 1) & 1))

        @pl.when(j < _BIG)
        def _():
            dsts = tuple(x.at[0, pl.ds(j, 1)] for x in (k_big, q_big, v_big))
            start_loads(big0 + j, 1, dsts, sem_bi.at[0])

        run([small(x, j) for x in (q_small, k_small, v_small, o_small)], j)

    jax.lax.fori_loop(0, _N_FIRST, first_step, None)
    start_loads(big0 + _BIG, _BIG, *big_in(1))
    first_out[0].start()

    def start_last_loads():
        for j in range(_N_LAST - 1):
            start_loads(last0 + _SMALL * j, _SMALL, *small_in(j, j))
        j = _N_LAST - 1
        head = n_heads - _SMALL
        sem = sem_si.at[j]
        copy(k_hbm.at[pl.ds(head + 1, _SMALL - 1)],
             k_small.at[pl.ds(_SMALL * j, _SMALL - 1)], sem).start()
        copy(k_hbm.at[n_heads - 1], k_small.at[_SMALL * j + _SMALL - 1], sem).start()
        copy(q_hbm.at[pl.ds(head, _SMALL)], small(q_small, j), sem).start()
        copy(v_hbm.at[pl.ds(head, _SMALL)], small(v_small, j), sem).start()

    def big_step(i, _):
        slot = i & 1
        wait_loads(*big_in(slot))

        @pl.when(i >= 2)
        def _():
            big_out(i - 2).wait()

        run([x.at[slot] for x in (q_big, k_big, v_big, o_big)], i)

        @pl.when(i + 2 < n_big)
        def _():
            start_loads(big0 + _BIG * (i + 2), _BIG, *big_in(slot))

        @pl.when(i + 2 == n_big)
        def _():
            start_last_loads()
            first_out[1].start()

        big_out(i).start()

    jax.lax.fori_loop(0, n_big, big_step, None)

    def last_step(j, _):
        wait_loads(*small_in(j, j))
        run([small(x, j) for x in (q_small, k_small, v_small)]
            + [small(o_small, _N_FIRST + j)], j)
        last_out(j).start()

    jax.lax.fori_loop(0, _N_LAST, last_step, None)

    first_out[0].wait()
    first_out[1].wait()
    big_out(n_big - 2).wait()
    big_out(n_big - 1).wait()
    for j in range(_N_LAST):
        last_out(j).wait()


@jax.jit
def pallas_standalone__gqa_softmax__near_ridge_kernel(
    q: jax.Array,
    k: jax.Array,
    v: jax.Array,
):
    B, Hq, Sq, D = q.shape
    Hkv, Sk = k.shape[1], k.shape[2]
    assert Hq == Hkv and D == 192 and Sk == 512
    n = B * Hq
    qt = jnp.swapaxes(q, 2, 3).reshape(n, 3, D // 3, Sq)
    kt = jnp.swapaxes(k, 2, 3).reshape(n, D, Sk)
    vt = jnp.swapaxes(v, 2, 3).reshape(n, D, Sk)

    def buffers(heads_in, heads_out):
        return [pltpu.VMEM((*heads_in, 3, D // 3, Sq), q.dtype),
                pltpu.VMEM((*heads_in, D, Sk), k.dtype),
                pltpu.VMEM((*heads_in, D, Sk), v.dtype),
                pltpu.VMEM((*heads_out, D, Sq), q.dtype)]

    ot = pl.pallas_call(
        functools.partial(_attn_kernel, scale_log2e=(D ** -0.5) * math.log2(math.e)),
        in_specs=[pl.BlockSpec(memory_space=pl.ANY)] * 3,
        out_specs=pl.BlockSpec(memory_space=pl.ANY),
        out_shape=jax.ShapeDtypeStruct((n, D, Sq), q.dtype),
        scratch_shapes=[
            *buffers((_SMALL * _N_FIRST,), (_SMALL * (_N_FIRST + _N_LAST),)),
            *buffers((2, _BIG), (2, _BIG)),
            pltpu.VMEM((3, 64, Sk // 2), _U32),
            pltpu.VMEM((3, Sk // 4, 128), _U32),
            pltpu.SemaphoreType.DMA((_N_LAST,)),
            pltpu.SemaphoreType.DMA((_N_LAST + 2,)),
            pltpu.SemaphoreType.DMA((2,)),
            pltpu.SemaphoreType.DMA((2,)),
            *[pltpu.VMEM((1, Sk, 128), _F32)] * _S_SLOTS,
        ],
        compiler_params=pltpu.CompilerParams(
            vmem_limit_bytes=100 * 1024 * 1024,
            disable_bounds_checks=True,
            flags={"XLA_TPU_FORCE_LP_LLO_SCHEDULER": True},
        ),
    )(qt, kt, vt)
    return jnp.swapaxes(ot.reshape(B, Hq, D, Sq), 2, 3)
```

```python
import functools
import math

import jax
import jax.numpy as jnp
import jax.experimental.pallas as pl
import jax.experimental.pallas.tpu as pltpu

_F32 = jnp.float32
_BF16 = jnp.bfloat16
_U32 = jnp.uint32

_BIG = 12
_SMALL = 2
_N_FIRST = 13
_N_LAST = 3
_PV_LAG = 3
_REM_POS = 3
_K_PREP_POS = 4
_S_SLOTS = 4


def _dot(a, b):
    return jnp.dot(a, b, preferred_element_type=_F32)


def _dot_tn(a, b):
    return jax.lax.dot_general(a, b, (((0,), (0,)), ((), ())), preferred_element_type=_F32)


def _dot_nt(a, b):
    return jax.lax.dot_general(a, b, (((1,), (1,)), ((), ())), preferred_element_type=_F32)


def _sum(xs):
    return functools.reduce(lambda a, b: a + b, xs)


def _reciprocal(x):
    r = pl.reciprocal(x, approx=True)
    return r * (2.0 - x * r)


def _prep_k(k_ref, scale_log2e):
    half = k_ref.shape[1] // 2

    def blk(r, col):
        x = k_ref[64 * r:64 * (r + 1), half * col:half * (col + 1)]
        return x.astype(_F32) * scale_log2e

    k1a, k1b, k1c = blk(0, 0), blk(1, 0), blk(2, 0)
    k2a, k2b, k2c = blk(0, 1), blk(1, 1), blk(2, 1)

    def cat(a, b):
        return jnp.concatenate([a, b], 0).astype(_BF16)

    kn = (cat(k1a, k2b), cat(k1b - k2b, k1c), cat(k2a - k1a, k2c))
    return kn, tuple(x.T for x in kn)


def _save_k(k, kn_ref, kt_ref):
    for j in range(3):
        kn_ref[j] = pltpu.bitcast(k[0][j], _U32)
        kt_ref[j] = pltpu.bitcast(k[1][j], _U32)


def _load_k(kn_ref, kt_ref):
    return (tuple(pltpu.bitcast(kn_ref[j], _BF16) for j in range(3)),
            tuple(pltpu.bitcast(kt_ref[j], _BF16) for j in range(3)))


def _group(q_ref, k_ref, v_ref, o_ref, kn_ref, kt_ref, s_refs, zero, scale_log2e):
    heads, _, sq = o_ref.shape
    sk = k_ref.shape[2]
    tiles = [(a, a + 128) for a in range(0, sq - 127, 128)]
    if sq % 128:
        tiles.insert(_REM_POS, (sq - sq % 128, sq))
    items = [(h, a, b) for h in range(heads) for a, b in tiles]
    full = [i for i, (_, a, b) in enumerate(items) if b - a == 128]
    s_ref = {i: s_refs[j % len(s_refs)] for j, i in enumerate(full)}
    ks = {0: _load_k(kn_ref, kt_ref)}
    vs, scores, probs = {}, {}, {}

    def qk(i):
        h, a, b = items[i]
        w = b - a
        q_ab = q_ref[h, 0:2, :, a:b].reshape(128, w)
        q_bc = q_ref[h, 1:3, :, a:b].reshape(128, w)
        q_ac = jnp.concatenate(
            [q_ref[h, 0:1, :, a:b], q_ref[h, 2:3, :, a:b]], 0).reshape(128, w)
        if w == 128:
            k1, k2, k3 = ks[h][1]
            t1 = _dot(k1, q_ab)
            s1 = t1 + _dot(k2, q_bc)
            s2 = t1 + _dot(k3, q_ac)
            scores[i] = jnp.max(jnp.maximum(s1, s2), axis=0, keepdims=True)
            s_ref[i][0, 0:sk // 2, :] = s1
            s_ref[i][0, sk // 2:sk, :] = s2
        else:
            k1, k2, k3 = ks[h][0]
            t1 = _dot_tn(q_ab, k1)
            s1 = t1 + _dot_tn(q_bc, k2)
            s2 = t1 + _dot_tn(q_ac, k3)
            scores[i] = (s1, s2, jnp.max(jnp.maximum(s1, s2), axis=1, keepdims=True))

    def softmax(i):
        _, a, b = items[i]
        w = b - a
        if w == 128:
            m = jnp.broadcast_to(scores.pop(i), (8, w))
            acc, es, p = None, [], []
            for r in range(0, sk, 8):
                e = jnp.exp2(s_ref[i][zero, r:r + 8, :] - m)
                acc = e if acc is None else acc + e
                es.append(e)
                if len(es) == 16:
                    p.append(jnp.concatenate(es, 0).astype(_BF16))
                    es = []
            probs[i] = (p, _reciprocal(jnp.sum(acc, axis=0, keepdims=True)))
        else:
            s1, s2, m = scores.pop(i)
            m = jnp.broadcast_to(m, (w, 128))
            es = [jnp.exp2(s[:, j:j + 128] - m)
                  for s in (s1, s2) for j in range(0, sk // 2, 128)]
            inv = _reciprocal(
                jnp.sum((es[0] + es[1]) + (es[2] + es[3]), axis=1, keepdims=True))
            probs[i] = ([e.astype(_BF16) for e in es], inv)

    def pv(i):
        h, a, b = items[i]
        if h not in vs:
            vs[h] = [(v_ref[h, 0:128, j:j + 128], v_ref[h, :, j:j + 128],
                      v_ref[h, 128:192, j:j + 128]) for j in range(0, sk, 128)]
        p, inv = probs.pop(i)
        if b - a == 128:
            o = _sum([_dot(v[1], pj) for v, pj in zip(vs[h], p)])
            o_ref[h, :, a:b] = (o * inv).astype(o_ref.dtype)
        else:
            o_lo = _sum([_dot_nt(pj, v[0]) for v, pj in zip(vs[h], p)])
            o_hi = _sum([_dot_nt(v[2], pj) for v, pj in zip(vs[h], p)])
            inv = jnp.broadcast_to(inv, (b - a, 128))
            o_lo = o_lo * inv
            o_hi = o_hi * inv.T[0:64]
            o_ref[h, 0:128, a:b] = o_lo.astype(o_ref.dtype).T
            o_ref[h, 128:192, a:b] = o_hi.astype(o_ref.dtype)

    n = len(items)
    for step in range(n + _PV_LAG):
        h, t = divmod(step, len(tiles))
        if step < n and t == _K_PREP_POS:
            ks[h + 1] = _prep_k(k_ref.at[h], scale_log2e)
            if h + 1 == heads:
                _save_k(ks[heads], kn_ref, kt_ref)
        if step < n:
            qk(step)
        if 0 <= step - 1 < n:
            softmax(step - 1)
        if 0 <= step - _PV_LAG:
            pv(step - _PV_LAG)


def _attn_kernel(q_hbm, k_hbm, v_hbm, o_hbm,
                 q_small, k_small, v_small, o_small, q_big, k_big, v_big, o_big,
                 kn_ref, kt_ref, sem_si, sem_so, sem_bi, sem_bo, *s_refs, scale_log2e):
    n_heads = q_hbm.shape[0]
    n_big = (n_heads - _SMALL * (_N_FIRST + _N_LAST)) // _BIG
    big0 = _SMALL * _N_FIRST
    last0 = big0 + _BIG * n_big
    assert last0 + _SMALL * _N_LAST == n_heads and n_big >= _N_FIRST
    assert _N_FIRST >= max(_BIG, _N_LAST) and _N_LAST >= 2
    copy = pltpu.make_async_copy

    def small(ref, j):
        return ref.at[pl.ds(_SMALL * j, _SMALL)]

    def start_loads(head, n, dsts, sem):
        for src, dst, off in zip((k_hbm, q_hbm, v_hbm), dsts, (1, 0, 0)):
            copy(src.at[pl.ds(head + off, n)], dst, sem).start()

    def wait_loads(dsts, sem):
        for dst in dsts:
            copy(dst, dst, sem).wait()

    def small_in(j, sem):
        return tuple(small(x, j) for x in (k_small, q_small, v_small)), sem_si.at[sem]

    def big_in(slot):
        return tuple(x.at[slot] for x in (k_big, q_big, v_big)), sem_bi.at[slot]

    def big_out(i):
        return copy(o_big.at[i & 1], o_hbm.at[pl.ds(big0 + _BIG * i, _BIG)], sem_bo.at[i & 1])

    def last_out(j):
        return copy(small(o_small, _N_FIRST + j),
                    o_hbm.at[pl.ds(last0 + _SMALL * j, _SMALL)], sem_so.at[j])

    def run(bufs, it):
        zero = jax.lax.shift_right_logical(it, 30)
        _group(*bufs, kn_ref, kt_ref, s_refs, zero, scale_log2e)

    k0 = copy(k_hbm.at[0], k_big.at[1, 0], sem_bi.at[1])
    k0.start()
    start_loads(0, _SMALL, *small_in(0, 0))
    k0.wait()
    _save_k(_prep_k(k_big.at[1, 0], scale_log2e), kn_ref, kt_ref)

    def first_step(j, _):
        wait_loads(*small_in(j, j & 1))

        @pl.when(j + 1 < _N_FIRST)
        def _():
            start_loads(_SMALL * (j + 1), _SMALL, *small_in(j + 1, (j + 1) & 1))

        @pl.when(j < _BIG)
        def _():
            dsts = tuple(x.at[0, pl.ds(j, 1)] for x in (k_big, q_big, v_big))
            start_loads(big0 + j, 1, dsts, sem_bi.at[0])

        run([small(x, j) for x in (q_small, k_small, v_small, o_small)], j)

    jax.lax.fori_loop(0, _N_FIRST, first_step, None)
    start_loads(big0 + _BIG, _BIG, *big_in(1))

    def big_step(i, _):
        slot = i & 1
        wait_loads(*big_in(slot))

        @pl.when(i >= 2)
        def _():
            big_out(i - 2).wait()

        run([x.at[slot] for x in (q_big, k_big, v_big, o_big)], i)

        @pl.when(i + 2 < n_big)
        def _():
            start_loads(big0 + _BIG * (i + 2), _BIG, *big_in(slot))

        big_out(i).start()

        @pl.when(i < _N_LAST)
        def _():
            head = last0 + _SMALL * i
            sem = sem_si.at[i]
            copy(k_hbm.at[pl.ds(head + 1, _SMALL - 1)],
                 k_small.at[pl.ds(_SMALL * i, _SMALL - 1)], sem).start()
            copy(k_hbm.at[jnp.minimum(head + _SMALL, n_heads - 1)],
                 k_small.at[_SMALL * i + _SMALL - 1], sem).start()
            copy(q_hbm.at[pl.ds(head, _SMALL)], small(q_small, i), sem).start()
            copy(v_hbm.at[pl.ds(head, _SMALL)], small(v_small, i), sem).start()

        @pl.when(i < _N_FIRST)
        def _():
            copy(small(o_small, i), small(o_hbm, i), sem_so.at[_N_LAST]).start()

    jax.lax.fori_loop(0, n_big, big_step, None)

    def last_step(j, _):
        wait_loads(*small_in(j, j))
        run([small(x, j) for x in (q_small, k_small, v_small)]
            + [small(o_small, _N_FIRST + j)], j)
        last_out(j).start()

    jax.lax.fori_loop(0, _N_LAST, last_step, None)

    copy(o_small.at[pl.ds(0, big0)], o_hbm.at[pl.ds(0, big0)], sem_so.at[_N_LAST]).wait()
    big_out(n_big - 2).wait()
    big_out(n_big - 1).wait()
    for j in range(_N_LAST):
        last_out(j).wait()


@jax.jit
def pallas_standalone__gqa_softmax__near_ridge_kernel(
    q: jax.Array,
    k: jax.Array,
    v: jax.Array,
):
    B, Hq, Sq, D = q.shape
    Hkv, Sk = k.shape[1], k.shape[2]
    assert Hq == Hkv and D == 192 and Sk == 512
    n = B * Hq
    qt = jnp.swapaxes(q, 2, 3).reshape(n, 3, D // 3, Sq)
    kt = jnp.swapaxes(k, 2, 3).reshape(n, D, Sk)
    vt = jnp.swapaxes(v, 2, 3).reshape(n, D, Sk)

    def buffers(heads_in, heads_out):
        return [pltpu.VMEM((*heads_in, 3, D // 3, Sq), q.dtype),
                pltpu.VMEM((*heads_in, D, Sk), k.dtype),
                pltpu.VMEM((*heads_in, D, Sk), v.dtype),
                pltpu.VMEM((*heads_out, D, Sq), q.dtype)]

    ot = pl.pallas_call(
        functools.partial(_attn_kernel, scale_log2e=(D ** -0.5) * math.log2(math.e)),
        in_specs=[pl.BlockSpec(memory_space=pl.ANY)] * 3,
        out_specs=pl.BlockSpec(memory_space=pl.ANY),
        out_shape=jax.ShapeDtypeStruct((n, D, Sq), q.dtype),
        scratch_shapes=[
            *buffers((_SMALL * _N_FIRST,), (_SMALL * (_N_FIRST + _N_LAST),)),
            *buffers((2, _BIG), (2, _BIG)),
            pltpu.VMEM((3, 64, Sk // 2), _U32),
            pltpu.VMEM((3, Sk // 4, 128), _U32),
            pltpu.SemaphoreType.DMA((_N_LAST,)),
            pltpu.SemaphoreType.DMA((_N_LAST + 1,)),
            pltpu.SemaphoreType.DMA((2,)),
            pltpu.SemaphoreType.DMA((2,)),
            *[pltpu.VMEM((1, Sk, 128), _F32)] * _S_SLOTS,
        ],
        compiler_params=pltpu.CompilerParams(
            vmem_limit_bytes=100 * 1024 * 1024,
            disable_bounds_checks=True,
            flags={"XLA_TPU_FORCE_LP_LLO_SCHEDULER": True},
        ),
    )(qt, kt, vt)
    return jnp.swapaxes(ot.reshape(B, Hq, D, Sq), 2, 3)
```

```python
import functools
import math

import jax
import jax.numpy as jnp
import jax.experimental.pallas as pl
import jax.experimental.pallas.tpu as pltpu

_F32 = jnp.float32
_BF16 = jnp.bfloat16
_U32 = jnp.uint32

_BIG = 12
_SMALL = 2
_N_FIRST = 13
_N_LAST = 3
_PV_LAG = 3
_REM_POS = 3
_K_PREP_POS = 4
_S_SLOTS = 4


def _dot(a, b):
    return jnp.dot(a, b, preferred_element_type=_F32)


def _dot_tn(a, b):
    return jax.lax.dot_general(a, b, (((0,), (0,)), ((), ())), preferred_element_type=_F32)


def _dot_nt(a, b):
    return jax.lax.dot_general(a, b, (((1,), (1,)), ((), ())), preferred_element_type=_F32)


def _sum(xs):
    return functools.reduce(lambda a, b: a + b, xs)


def _reciprocal(x):
    r = pl.reciprocal(x, approx=True)
    return r * (2.0 - x * r)


def _prep_k(k_ref, scale_log2e):
    half = k_ref.shape[1] // 2

    def blk(r, col):
        x = k_ref[64 * r:64 * (r + 1), half * col:half * (col + 1)]
        return x.astype(_F32) * scale_log2e

    k1a, k1b, k1c = blk(0, 0), blk(1, 0), blk(2, 0)
    k2a, k2b, k2c = blk(0, 1), blk(1, 1), blk(2, 1)

    def cat(a, b):
        return jnp.concatenate([a, b], 0).astype(_BF16)

    kn = (cat(k1a, k2b), cat(k1b - k2b, k1c), cat(k2a - k1a, k2c))
    return kn, tuple(x.T for x in kn)


def _save_k(k, kn_ref, kt_ref):
    for j in range(3):
        kn_ref[j] = pltpu.bitcast(k[0][j], _U32)
        kt_ref[j] = pltpu.bitcast(k[1][j], _U32)


def _load_k(kn_ref, kt_ref):
    return (tuple(pltpu.bitcast(kn_ref[j], _BF16) for j in range(3)),
            tuple(pltpu.bitcast(kt_ref[j], _BF16) for j in range(3)))


def _group(q_ref, k_ref, v_ref, o_ref, kn_ref, kt_ref, s_refs, zero, scale_log2e):
    heads, _, sq = o_ref.shape
    sk = k_ref.shape[2]
    tiles = [(a, a + 128) for a in range(0, sq - 127, 128)]
    if sq % 128:
        tiles.insert(_REM_POS, (sq - sq % 128, sq))
    items = [(h, a, b) for h in range(heads) for a, b in tiles]
    full = [i for i, (_, a, b) in enumerate(items) if b - a == 128]
    s_ref = {i: s_refs[j % len(s_refs)] for j, i in enumerate(full)}
    ks = {0: _load_k(kn_ref, kt_ref)}
    vs, scores, probs = {}, {}, {}

    def qk(i):
        h, a, b = items[i]
        w = b - a
        q_ab = q_ref[h, 0:2, :, a:b].reshape(128, w)
        q_bc = q_ref[h, 1:3, :, a:b].reshape(128, w)
        q_ac = jnp.concatenate(
            [q_ref[h, 0:1, :, a:b], q_ref[h, 2:3, :, a:b]], 0).reshape(128, w)
        if w == 128:
            k1, k2, k3 = ks[h][1]
            t1 = _dot(k1, q_ab)
            s1 = t1 + _dot(k2, q_bc)
            s2 = t1 + _dot(k3, q_ac)
            scores[i] = jnp.max(jnp.maximum(s1, s2), axis=0, keepdims=True)
            s_ref[i][0, 0:sk // 2, :] = s1
            s_ref[i][0, sk // 2:sk, :] = s2
        else:
            k1, k2, k3 = ks[h][0]
            t1 = _dot_tn(q_ab, k1)
            s1 = t1 + _dot_tn(q_bc, k2)
            s2 = t1 + _dot_tn(q_ac, k3)
            scores[i] = (s1, s2, jnp.max(jnp.maximum(s1, s2), axis=1, keepdims=True))

    def softmax(i):
        _, a, b = items[i]
        w = b - a
        if w == 128:
            m = jnp.broadcast_to(scores.pop(i), (8, w))
            acc, es, p = None, [], []
            for r in range(0, sk, 8):
                e = jnp.exp2(s_ref[i][zero, r:r + 8, :] - m)
                acc = e if acc is None else acc + e
                es.append(e)
                if len(es) == 16:
                    p.append(jnp.concatenate(es, 0).astype(_BF16))
                    es = []
            probs[i] = (p, _reciprocal(jnp.sum(acc, axis=0, keepdims=True)))
        else:
            s1, s2, m = scores.pop(i)
            m = jnp.broadcast_to(m, (w, 128))
            es = [jnp.exp2(s[:, j:j + 128] - m)
                  for s in (s1, s2) for j in range(0, sk // 2, 128)]
            inv = _reciprocal(
                jnp.sum((es[0] + es[1]) + (es[2] + es[3]), axis=1, keepdims=True))
            probs[i] = ([e.astype(_BF16) for e in es], inv)

    def pv(i):
        h, a, b = items[i]
        if h not in vs:
            vs[h] = [(v_ref[h, 0:128, j:j + 128], v_ref[h, :, j:j + 128],
                      v_ref[h, 128:192, j:j + 128]) for j in range(0, sk, 128)]
        p, inv = probs.pop(i)
        if b - a == 128:
            o = _sum([_dot(v[1], pj) for v, pj in zip(vs[h], p)])
            o_ref[h, :, a:b] = (o * inv).astype(o_ref.dtype)
        else:
            o_lo = _sum([_dot_nt(pj, v[0]) for v, pj in zip(vs[h], p)])
            o_hi = _sum([_dot_nt(v[2], pj) for v, pj in zip(vs[h], p)])
            inv = jnp.broadcast_to(inv, (b - a, 128))
            o_lo = o_lo * inv
            o_hi = o_hi * inv.T[0:64]
            o_ref[h, 0:128, a:b] = o_lo.astype(o_ref.dtype).T
            o_ref[h, 128:192, a:b] = o_hi.astype(o_ref.dtype)

    n = len(items)
    for step in range(n + _PV_LAG):
        h, t = divmod(step, len(tiles))
        if step < n and t == _K_PREP_POS:
            ks[h + 1] = _prep_k(k_ref.at[h], scale_log2e)
            if h + 1 == heads:
                _save_k(ks[heads], kn_ref, kt_ref)
        if step < n:
            qk(step)
        if 0 <= step - 1 < n:
            softmax(step - 1)
        if 0 <= step - _PV_LAG:
            pv(step - _PV_LAG)


def _attn_kernel(q_hbm, k_hbm, v_hbm, o_hbm,
                 q_small, k_small, v_small, o_small, q_big, k_big, v_big, o_big,
                 kn_ref, kt_ref, sem_si, sem_so, sem_bi, sem_bo, *s_refs, scale_log2e):
    n_heads = q_hbm.shape[0]
    n_big = (n_heads - _SMALL * (_N_FIRST + _N_LAST)) // _BIG
    big0 = _SMALL * _N_FIRST
    last0 = big0 + _BIG * n_big
    last_load_quad = _N_FIRST // 4 + 2
    assert last0 + _SMALL * _N_LAST == n_heads
    assert n_big >= 4 * (last_load_quad + _N_LAST)
    assert _N_FIRST >= max(_BIG, _N_LAST) and _N_LAST >= 2
    copy = pltpu.make_async_copy

    def small(ref, j):
        return ref.at[pl.ds(_SMALL * j, _SMALL)]

    def start_loads(head, n, dsts, sem):
        for src, dst, off in zip((k_hbm, q_hbm, v_hbm), dsts, (1, 0, 0)):
            copy(src.at[pl.ds(head + off, n)], dst, sem).start()

    def wait_loads(dsts, sem):
        for dst in dsts:
            copy(dst, dst, sem).wait()

    def small_in(j, sem):
        return tuple(small(x, j) for x in (k_small, q_small, v_small)), sem_si.at[sem]

    def big_in(slot):
        return tuple(x.at[slot] for x in (k_big, q_big, v_big)), sem_bi.at[slot]

    def big_out(i):
        return copy(o_big.at[i & 1], o_hbm.at[pl.ds(big0 + _BIG * i, _BIG)], sem_bo.at[i & 1])

    def last_out(j):
        return copy(small(o_small, _N_FIRST + j),
                    o_hbm.at[pl.ds(last0 + _SMALL * j, _SMALL)], sem_so.at[j])

    def run(bufs, it):
        zero = jax.lax.shift_right_logical(it, 30)
        _group(*bufs, kn_ref, kt_ref, s_refs, zero, scale_log2e)

    k0 = copy(k_hbm.at[0], k_big.at[1, 0], sem_bi.at[1])
    k0.start()
    start_loads(0, _SMALL, *small_in(0, 0))
    k0.wait()
    _save_k(_prep_k(k_big.at[1, 0], scale_log2e), kn_ref, kt_ref)

    def first_step(j, _):
        wait_loads(*small_in(j, j & 1))

        @pl.when(j + 1 < _N_FIRST)
        def _():
            start_loads(_SMALL * (j + 1), _SMALL, *small_in(j + 1, (j + 1) & 1))

        @pl.when(j < _BIG)
        def _():
            dsts = tuple(x.at[0, pl.ds(j, 1)] for x in (k_big, q_big, v_big))
            start_loads(big0 + j, 1, dsts, sem_bi.at[0])

        run([small(x, j) for x in (q_small, k_small, v_small, o_small)], j)

    jax.lax.fori_loop(0, _N_FIRST, first_step, None)
    start_loads(big0 + _BIG, _BIG, *big_in(1))

    def big_step(i, _):
        slot = i & 1
        wait_loads(*big_in(slot))

        @pl.when(i >= 2)
        def _():
            big_out(i - 2).wait()

        run([x.at[slot] for x in (q_big, k_big, v_big, o_big)], i)

        @pl.when(i + 2 < n_big)
        def _():
            start_loads(big0 + _BIG * (i + 2), _BIG, *big_in(slot))

        big_out(i).start()

        @pl.when(i < _N_FIRST)
        def _():
            copy(small(o_small, i), small(o_hbm, i), sem_so.at[_N_LAST]).start()

        j = (i >> 2) - last_load_quad

        @pl.when((j >= 0) & (j < _N_LAST) & (i & 3 == 0))
        def _():
            head = last0 + _SMALL * j
            sem = sem_si.at[j]
            copy(k_hbm.at[pl.ds(head + 1, _SMALL - 1)],
                 k_small.at[pl.ds(_SMALL * j, _SMALL - 1)], sem).start()
            copy(k_hbm.at[jnp.minimum(head + _SMALL, n_heads - 1)],
                 k_small.at[_SMALL * j + _SMALL - 1], sem).start()
            copy(q_hbm.at[pl.ds(head, _SMALL)], small(q_small, j), sem).start()
            copy(v_hbm.at[pl.ds(head, _SMALL)], small(v_small, j), sem).start()

    jax.lax.fori_loop(0, n_big, big_step, None)

    def last_step(j, _):
        wait_loads(*small_in(j, j))
        run([small(x, j) for x in (q_small, k_small, v_small)]
            + [small(o_small, _N_FIRST + j)], j)
        last_out(j).start()

    jax.lax.fori_loop(0, _N_LAST, last_step, None)

    copy(o_small.at[pl.ds(0, big0)], o_hbm.at[pl.ds(0, big0)], sem_so.at[_N_LAST]).wait()
    big_out(n_big - 2).wait()
    big_out(n_big - 1).wait()
    for j in range(_N_LAST):
        last_out(j).wait()


@jax.jit
def pallas_standalone__gqa_softmax__near_ridge_kernel(
    q: jax.Array,
    k: jax.Array,
    v: jax.Array,
):
    B, Hq, Sq, D = q.shape
    Hkv, Sk = k.shape[1], k.shape[2]
    assert Hq == Hkv and D == 192 and Sk == 512
    n = B * Hq
    qt = jnp.swapaxes(q, 2, 3).reshape(n, 3, D // 3, Sq)
    kt = jnp.swapaxes(k, 2, 3).reshape(n, D, Sk)
    vt = jnp.swapaxes(v, 2, 3).reshape(n, D, Sk)

    def buffers(heads_in, heads_out):
        return [pltpu.VMEM((*heads_in, 3, D // 3, Sq), q.dtype),
                pltpu.VMEM((*heads_in, D, Sk), k.dtype),
                pltpu.VMEM((*heads_in, D, Sk), v.dtype),
                pltpu.VMEM((*heads_out, D, Sq), q.dtype)]

    ot = pl.pallas_call(
        functools.partial(_attn_kernel, scale_log2e=(D ** -0.5) * math.log2(math.e)),
        in_specs=[pl.BlockSpec(memory_space=pl.ANY)] * 3,
        out_specs=pl.BlockSpec(memory_space=pl.ANY),
        out_shape=jax.ShapeDtypeStruct((n, D, Sq), q.dtype),
        scratch_shapes=[
            *buffers((_SMALL * _N_FIRST,), (_SMALL * (_N_FIRST + _N_LAST),)),
            *buffers((2, _BIG), (2, _BIG)),
            pltpu.VMEM((3, 64, Sk // 2), _U32),
            pltpu.VMEM((3, Sk // 4, 128), _U32),
            pltpu.SemaphoreType.DMA((_N_LAST,)),
            pltpu.SemaphoreType.DMA((_N_LAST + 1,)),
            pltpu.SemaphoreType.DMA((2,)),
            pltpu.SemaphoreType.DMA((2,)),
            *[pltpu.VMEM((1, Sk, 128), _F32)] * _S_SLOTS,
        ],
        compiler_params=pltpu.CompilerParams(
            vmem_limit_bytes=100 * 1024 * 1024,
            disable_bounds_checks=True,
            flags={"XLA_TPU_FORCE_LP_LLO_SCHEDULER": True},
        ),
    )(qt, kt, vt)
    return jnp.swapaxes(ot.reshape(B, Hq, D, Sq), 2, 3)
```

```python
import functools
import math

import jax
import jax.numpy as jnp
import jax.experimental.pallas as pl
import jax.experimental.pallas.tpu as pltpu

_F32 = jnp.float32
_BF16 = jnp.bfloat16
_U32 = jnp.uint32

_BIG = 12
_SMALL = 2
_N_FIRST = 13
_N_LAST = 3
_PV_LAG = 3
_REM_POS = 3
_K_PREP_POS = 4
_S_SLOTS = 4
_GUARD = 8.0


def _dot(a, b):
    return jnp.dot(a, b, preferred_element_type=_F32)


def _dot_tn(a, b):
    return jax.lax.dot_general(a, b, (((0,), (0,)), ((), ())), preferred_element_type=_F32)


def _dot_nt(a, b):
    return jax.lax.dot_general(a, b, (((1,), (1,)), ((), ())), preferred_element_type=_F32)


def _sum(xs):
    return functools.reduce(lambda a, b: a + b, xs)


def _reciprocal(x):
    r = pl.reciprocal(x, approx=True)
    return r * (2.0 - x * r)


def _norm2(x):
    return jnp.sum(x * x, axis=0, keepdims=True)


def _prep_k(k_ref):
    half = k_ref.shape[1] // 2

    def blk(r, col):
        return k_ref[64 * r:64 * (r + 1), half * col:half * (col + 1)].astype(_F32)

    k1a, k1b, k1c = blk(0, 0), blk(1, 0), blk(2, 0)
    k2a, k2b, k2c = blk(0, 1), blk(1, 1), blk(2, 1)

    def cat(a, b):
        return jnp.concatenate([a, b], 0).astype(_BF16)

    da, db = k2a - k1a, k1b - k2b
    kn = (cat(k1a, k2b), cat(db, k1c), cat(da, k2c))
    kd = tuple(jnp.broadcast_to(jnp.max(_norm2(d), axis=1, keepdims=True), (1, 128))
               for d in (da, db))
    return kn, tuple(x.T for x in kn), kd


def _save_k(k, kn_ref, kt_ref, kd_ref):
    for j in range(3):
        kn_ref[j] = pltpu.bitcast(k[0][j], _U32)
        kt_ref[j] = pltpu.bitcast(k[1][j], _U32)
    for j in range(2):
        kd_ref[j] = k[2][j]


def _load_k(kn_ref, kt_ref, kd_ref):
    return (tuple(pltpu.bitcast(kn_ref[j], _BF16) for j in range(3)),
            tuple(pltpu.bitcast(kt_ref[j], _BF16) for j in range(3)),
            tuple(kd_ref[j] for j in range(2)))


def _head_exact(q_ref, k_ref, v_ref, o_ref, scale_log2e):
    s = _dot_tn(k_ref[...], q_ref[...].reshape(o_ref.shape))
    e = jnp.exp2((s - jnp.max(s, axis=0, keepdims=True)) * scale_log2e)
    o = _dot(v_ref[...], e.astype(_BF16)) / jnp.sum(e, axis=0, keepdims=True)
    o_ref[...] = o.astype(o_ref.dtype)


def _group(q_ref, k_ref, v_ref, o_ref, k_carry, s_refs, redo_ref, head0, zero, scale_log2e):
    heads, d, sq = o_ref.shape
    sk = k_ref.shape[2]
    tiles = [(a, a + 128) for a in range(0, sq - 127, 128)]
    if sq % 128:
        tiles.insert(_REM_POS, (sq - sq % 128, sq))
    items = [(h, a, b) for h in range(heads) for a, b in tiles]
    full = [i for i, (_, a, b) in enumerate(items) if b - a == 128]
    s_ref = {i: s_refs[j % len(s_refs)] for j, i in enumerate(full)}
    ks = {0: _load_k(*k_carry)}
    vs, scores, probs = {}, {}, {}

    def qk(i):
        h, a, b = items[i]
        w = b - a
        q_ab = q_ref[h, 0:2, :, a:b].reshape(128, w)
        q_bc = q_ref[h, 1:3, :, a:b].reshape(128, w)
        q_ac = jnp.concatenate(
            [q_ref[h, 0:1, :, a:b], q_ref[h, 2:3, :, a:b]], 0).reshape(128, w)
        if w == 128:
            k1, k2, k3 = ks[h][1]
            t1 = _dot(k1, q_ab)
            s1 = t1 + _dot(k2, q_bc)
            s2 = t1 + _dot(k3, q_ac)
            scores[i] = jnp.max(jnp.maximum(s1, s2), axis=0, keepdims=True)
            s_ref[i][0, 0:sk // 2, :] = s1
            s_ref[i][0, sk // 2:sk, :] = s2
        else:
            k1, k2, k3 = ks[h][0]
            t1 = _dot_tn(q_ab, k1)
            s1 = t1 + _dot_tn(q_bc, k2)
            s2 = t1 + _dot_tn(q_ac, k3)
            scores[i] = (s1, s2, jnp.max(jnp.maximum(s1, s2), axis=1, keepdims=True))

    def guard(i, m):
        h, a, b = items[i]
        limit = jnp.maximum(m * m, float(d)) * _GUARD ** 2
        ok_a, ok_b = (_norm2(q_ref[h, r, :, a:b].astype(_F32)) * ks[h][2][r][:, 0:b - a] < limit
                      for r in range(2))
        redo_ref[head0 + h, a // 128:a // 128 + 1, 0:b - a] = jnp.where(ok_a & ok_b, 0.0, 1.0)

    def softmax(i):
        _, a, b = items[i]
        w = b - a
        if w == 128:
            guard(i, scores[i])
            m = jnp.broadcast_to(scores.pop(i), (8, w))
            acc, es, p = None, [], []
            for r in range(0, sk, 8):
                e = jnp.exp2((s_ref[i][zero, r:r + 8, :] - m) * scale_log2e)
                acc = e if acc is None else acc + e
                es.append(e)
                if len(es) == 16:
                    p.append(jnp.concatenate(es, 0).astype(_BF16))
                    es = []
            probs[i] = (p, _reciprocal(jnp.sum(acc, axis=0, keepdims=True)))
        else:
            s1, s2, m = scores.pop(i)
            m = jnp.broadcast_to(m, (w, 128))
            es = [jnp.exp2((s[:, j:j + 128] - m) * scale_log2e)
                  for s in (s1, s2) for j in range(0, sk // 2, 128)]
            inv = _reciprocal(
                jnp.sum((es[0] + es[1]) + (es[2] + es[3]), axis=1, keepdims=True))
            inv = jnp.broadcast_to(inv, (w, 128))
            lane = jax.lax.broadcasted_iota(jnp.int32, (w, 128), 1)
            both_t = jnp.where(lane < 64, inv, m).T
            guard(i, both_t[64:65])
            probs[i] = ([e.astype(_BF16) for e in es], (inv, both_t[0:64]))

    def pv(i):
        h, a, b = items[i]
        if h not in vs:
            vs[h] = [(v_ref[h, 0:128, j:j + 128], v_ref[h, :, j:j + 128],
                      v_ref[h, 128:192, j:j + 128]) for j in range(0, sk, 128)]
        p, inv = probs.pop(i)
        if b - a == 128:
            o = _sum([_dot(v[1], pj) for v, pj in zip(vs[h], p)])
            o_ref[h, :, a:b] = (o * inv).astype(o_ref.dtype)
        else:
            o_lo = _sum([_dot_nt(pj, v[0]) for v, pj in zip(vs[h], p)])
            o_hi = _sum([_dot_nt(v[2], pj) for v, pj in zip(vs[h], p)])
            o_lo = o_lo * inv[0]
            o_hi = o_hi * inv[1]
            o_ref[h, 0:128, a:b] = o_lo.astype(o_ref.dtype).T
            o_ref[h, 128:192, a:b] = o_hi.astype(o_ref.dtype)

    n = len(items)
    for step in range(n + _PV_LAG):
        h, t = divmod(step, len(tiles))
        if step < n and t == _K_PREP_POS:
            ks[h + 1] = _prep_k(k_ref.at[h])
            if h + 1 == heads:
                _save_k(ks[heads], *k_carry)
        if step < n:
            qk(step)
        if 0 <= step - 1 < n:
            softmax(step - 1)
        if 0 <= step - _PV_LAG:
            pv(step - _PV_LAG)


def _attn_kernel(q_hbm, k_hbm, v_hbm, o_hbm,
                 q_small, k_small, v_small, o_small, q_big, k_big, v_big, o_big,
                 kn_ref, kt_ref, kd_ref, redo_ref,
                 sem_si, sem_so, sem_bi, sem_bo, *s_refs, scale_log2e):
    k_carry = (kn_ref, kt_ref, kd_ref)
    n_heads = q_hbm.shape[0]
    n_big = (n_heads - _SMALL * (_N_FIRST + _N_LAST)) // _BIG
    big0 = _SMALL * _N_FIRST
    last0 = big0 + _BIG * n_big
    last_load_quad = _N_FIRST // 4 + 2
    assert last0 + _SMALL * _N_LAST == n_heads
    assert n_big >= 4 * (last_load_quad + _N_LAST)
    assert _N_FIRST >= max(_BIG, _N_LAST) and _N_LAST >= 2
    copy = pltpu.make_async_copy

    def small(ref, j):
        return ref.at[pl.ds(_SMALL * j, _SMALL)]

    def start_loads(head, n, dsts, sem):
        for src, dst, off in zip((k_hbm, q_hbm, v_hbm), dsts, (1, 0, 0)):
            copy(src.at[pl.ds(head + off, n)], dst, sem).start()

    def wait_loads(dsts, sem):
        for dst in dsts:
            copy(dst, dst, sem).wait()

    def small_in(j, sem):
        return tuple(small(x, j) for x in (k_small, q_small, v_small)), sem_si.at[sem]

    def big_in(slot):
        return tuple(x.at[slot] for x in (k_big, q_big, v_big)), sem_bi.at[slot]

    def big_out(i):
        return copy(o_big.at[i & 1], o_hbm.at[pl.ds(big0 + _BIG * i, _BIG)], sem_bo.at[i & 1])

    def last_out(j):
        return copy(small(o_small, _N_FIRST + j),
                    o_hbm.at[pl.ds(last0 + _SMALL * j, _SMALL)], sem_so.at[j])

    def run(bufs, head0):
        zero = jax.lax.shift_right_logical(head0, 30)
        _group(*bufs, k_carry, s_refs, redo_ref, head0, zero, scale_log2e)

    k0 = copy(k_hbm.at[0], k_big.at[1, 0], sem_bi.at[1])
    k0.start()
    start_loads(0, _SMALL, *small_in(0, 0))
    redo_ref[...] = jnp.zeros(redo_ref.shape, _F32)
    k0.wait()
    _save_k(_prep_k(k_big.at[1, 0]), *k_carry)

    def first_step(j, _):
        wait_loads(*small_in(j, j & 1))

        @pl.when(j + 1 < _N_FIRST)
        def _():
            start_loads(_SMALL * (j + 1), _SMALL, *small_in(j + 1, (j + 1) & 1))

        @pl.when(j < _BIG)
        def _():
            dsts = tuple(x.at[0, pl.ds(j, 1)] for x in (k_big, q_big, v_big))
            start_loads(big0 + j, 1, dsts, sem_bi.at[0])

        run([small(x, j) for x in (q_small, k_small, v_small, o_small)], _SMALL * j)

    jax.lax.fori_loop(0, _N_FIRST, first_step, None)
    start_loads(big0 + _BIG, _BIG, *big_in(1))

    def big_step(i, _):
        slot = i & 1
        wait_loads(*big_in(slot))

        @pl.when(i >= 2)
        def _():
            big_out(i - 2).wait()

        run([x.at[slot] for x in (q_big, k_big, v_big, o_big)], big0 + _BIG * i)

        @pl.when(i + 2 < n_big)
        def _():
            start_loads(big0 + _BIG * (i + 2), _BIG, *big_in(slot))

        big_out(i).start()

        @pl.when(i < _N_FIRST)
        def _():
            copy(small(o_small, i), small(o_hbm, i), sem_so.at[_N_LAST]).start()

        j = (i >> 2) - last_load_quad

        @pl.when((j >= 0) & (j < _N_LAST) & (i & 3 == 0))
        def _():
            head = last0 + _SMALL * j
            sem = sem_si.at[j]
            copy(k_hbm.at[pl.ds(head + 1, _SMALL - 1)],
                 k_small.at[pl.ds(_SMALL * j, _SMALL - 1)], sem).start()
            copy(k_hbm.at[jnp.minimum(head + _SMALL, n_heads - 1)],
                 k_small.at[_SMALL * j + _SMALL - 1], sem).start()
            copy(q_hbm.at[pl.ds(head, _SMALL)], small(q_small, j), sem).start()
            copy(v_hbm.at[pl.ds(head, _SMALL)], small(v_small, j), sem).start()

    jax.lax.fori_loop(0, n_big, big_step, None)

    def last_step(j, _):
        wait_loads(*small_in(j, j))
        run([small(x, j) for x in (q_small, k_small, v_small)]
            + [small(o_small, _N_FIRST + j)], last0 + _SMALL * j)
        last_out(j).start()

    jax.lax.fori_loop(0, _N_LAST, last_step, None)
    any_redo = jnp.max(jnp.max(redo_ref[...], axis=0)) > 0.0

    copy(o_small.at[pl.ds(0, big0)], o_hbm.at[pl.ds(0, big0)], sem_so.at[_N_LAST]).wait()
    big_out(n_big - 2).wait()
    big_out(n_big - 1).wait()
    for j in range(_N_LAST):
        last_out(j).wait()

    def redo_step(head, _):
        @pl.when(jnp.max(redo_ref[head]) > 0.0)
        def _():
            q, k, v, o = (x.at[0, 0] for x in (q_big, k_big, v_big, o_big))
            for src, dst in ((q_hbm, q), (k_hbm, k), (v_hbm, v)):
                copy(src.at[head], dst, sem_bi.at[0]).start()
            wait_loads((q, k, v), sem_bi.at[0])
            _head_exact(q, k, v, o, scale_log2e)
            out = copy(o, o_hbm.at[head], sem_bo.at[0])
            out.start()
            out.wait()

    @pl.when(any_redo)
    def _():
        jax.lax.fori_loop(0, n_heads, redo_step, None)


@jax.jit
def pallas_standalone__gqa_softmax__near_ridge_kernel(
    q: jax.Array,
    k: jax.Array,
    v: jax.Array,
):
    B, Hq, Sq, D = q.shape
    Hkv, Sk = k.shape[1], k.shape[2]
    assert Hq == Hkv and D == 192 and Sk == 512 and Sq <= 8 * 128
    n = B * Hq
    qt = jnp.swapaxes(q, 2, 3).reshape(n, 3, D // 3, Sq)
    kt = jnp.swapaxes(k, 2, 3).reshape(n, D, Sk)
    vt = jnp.swapaxes(v, 2, 3).reshape(n, D, Sk)

    def buffers(heads_in, heads_out):
        return [pltpu.VMEM((*heads_in, 3, D // 3, Sq), q.dtype),
                pltpu.VMEM((*heads_in, D, Sk), k.dtype),
                pltpu.VMEM((*heads_in, D, Sk), v.dtype),
                pltpu.VMEM((*heads_out, D, Sq), q.dtype)]

    ot = pl.pallas_call(
        functools.partial(_attn_kernel, scale_log2e=(D ** -0.5) * math.log2(math.e)),
        in_specs=[pl.BlockSpec(memory_space=pl.ANY)] * 3,
        out_specs=pl.BlockSpec(memory_space=pl.ANY),
        out_shape=jax.ShapeDtypeStruct((n, D, Sq), q.dtype),
        scratch_shapes=[
            *buffers((_SMALL * _N_FIRST,), (_SMALL * (_N_FIRST + _N_LAST),)),
            *buffers((2, _BIG), (2, _BIG)),
            pltpu.VMEM((3, 64, Sk // 2), _U32),
            pltpu.VMEM((3, Sk // 4, 128), _U32),
            pltpu.VMEM((2, 1, 128), _F32),
            pltpu.VMEM((n, 8, 128), _F32),
            pltpu.SemaphoreType.DMA((_N_LAST,)),
            pltpu.SemaphoreType.DMA((_N_LAST + 1,)),
            pltpu.SemaphoreType.DMA((2,)),
            pltpu.SemaphoreType.DMA((2,)),
            *[pltpu.VMEM((1, Sk, 128), _F32)] * _S_SLOTS,
        ],
        compiler_params=pltpu.CompilerParams(
            vmem_limit_bytes=100 * 1024 * 1024,
            disable_bounds_checks=True,
            flags={"XLA_TPU_FORCE_LP_LLO_SCHEDULER": True},
        ),
    )(qt, kt, vt)
    return jnp.swapaxes(ot.reshape(B, Hq, D, Sq), 2, 3)
```

```python
import functools
import math

import jax
import jax.numpy as jnp
import jax.experimental.pallas as pl
import jax.experimental.pallas.tpu as pltpu

_F32 = jnp.float32
_BF16 = jnp.bfloat16
_U32 = jnp.uint32
_LOG2E = math.log2(math.e)

_BIG = 12
_SMALL = 2
_N_FIRST = 13
_N_LAST = 3
_PV_LAG = 3
_REM_POS = 3
_K_PREP_POS = 4
_S_SLOTS = 4
_GUARD = 8.0


def _dot(a, b):
    return jnp.dot(a, b, preferred_element_type=_F32)


def _dot_tn(a, b):
    return jax.lax.dot_general(a, b, (((0,), (0,)), ((), ())), preferred_element_type=_F32)


def _dot_nt(a, b):
    return jax.lax.dot_general(a, b, (((1,), (1,)), ((), ())), preferred_element_type=_F32)


def _sum(xs):
    return functools.reduce(lambda a, b: a + b, xs)


def _reciprocal(x):
    r = pl.reciprocal(x, approx=True)
    return r * (2.0 - x * r)


def _norm2(x, axis):
    return jnp.sum(x * x, axis=axis, keepdims=True)


def _prep_k(k_ref):
    half = k_ref.shape[1] // 2

    def blk(r, col):
        return k_ref[64 * r:64 * (r + 1), half * col:half * (col + 1)].astype(_F32)

    k1a, k1b, k1c = blk(0, 0), blk(1, 0), blk(2, 0)
    k2a, k2b, k2c = blk(0, 1), blk(1, 1), blk(2, 1)

    def cat(a, b):
        return jnp.concatenate([a, b], 0).astype(_BF16)

    da, db = k2a - k1a, k1b - k2b
    kn = (cat(k1a, k2b), cat(db, k1c), cat(da, k2c))
    kd = jnp.max(jnp.maximum(_norm2(da, 0), _norm2(db, 0)), axis=1, keepdims=True)
    return kn, tuple(x.T for x in kn), jnp.broadcast_to(kd, (1, 128))


def _save_k(k, kn_ref, kt_ref, kd_ref):
    for j in range(3):
        kn_ref[j] = pltpu.bitcast(k[0][j], _U32)
        kt_ref[j] = pltpu.bitcast(k[1][j], _U32)
    kd_ref[...] = k[2]


def _load_k(kn_ref, kt_ref, kd_ref):
    return (tuple(pltpu.bitcast(kn_ref[j], _BF16) for j in range(3)),
            tuple(pltpu.bitcast(kt_ref[j], _BF16) for j in range(3)),
            kd_ref[...])


def _head_exact(q_ref, k_ref, v_ref, o_ref, scale_log2e):
    s = _dot_tn(k_ref[...], q_ref[...].reshape(o_ref.shape))
    e = jnp.exp2((s - jnp.max(s, axis=0, keepdims=True)) * scale_log2e)
    o = _dot(v_ref[...], e.astype(_BF16)) / jnp.sum(e, axis=0, keepdims=True)
    o_ref[...] = o.astype(o_ref.dtype)


def _group(q_ref, k_ref, v_ref, o_ref, k_carry, s_refs, redo_ref, head0, zero, scale_log2e):
    heads, _, sq = o_ref.shape
    sk = k_ref.shape[2]
    tiles = [(a, a + 128) for a in range(0, sq - 127, 128)]
    if sq % 128:
        tiles.insert(_REM_POS, (sq - sq % 128, sq))
    items = [(h, a, b) for h in range(heads) for a, b in tiles]
    full = [i for i, (_, a, b) in enumerate(items) if b - a == 128]
    s_ref = {i: s_refs[j % len(s_refs)] for j, i in enumerate(full)}
    ks = {0: _load_k(*k_carry)}
    vs, scores, probs = {}, {}, {}

    def guarded_max(i, s1, s2, q_ab, axis):
        h, a, _ = items[i]
        m = jnp.max(jnp.maximum(s1, s2), axis=axis, keepdims=True)
        limit = jnp.maximum(m * m, _LOG2E ** 2) * (_GUARD / scale_log2e) ** 2
        flag = jnp.where(_norm2(q_ab.astype(_F32), axis) * ks[h][2] < limit, 0.0, 1.0)
        redo_ref[head0 + h, a // 128:a // 128 + 1, :] = jnp.max(flag, axis=0, keepdims=True)
        return m + flag

    def qk(i):
        h, a, b = items[i]
        w = b - a
        q_ab = q_ref[h, 0:2, :, a:b].reshape(128, w)
        q_bc = q_ref[h, 1:3, :, a:b].reshape(128, w)
        q_ac = jnp.concatenate(
            [q_ref[h, 0:1, :, a:b], q_ref[h, 2:3, :, a:b]], 0).reshape(128, w)
        if w == 128:
            k1, k2, k3 = ks[h][1]
            t1 = _dot(k1, q_ab)
            s1 = (t1 + _dot(k2, q_bc)) * scale_log2e
            s2 = (t1 + _dot(k3, q_ac)) * scale_log2e
            scores[i] = guarded_max(i, s1, s2, q_ref[h, 0:2, :, a:b].reshape(128, w), 0)
            s_ref[i][0, 0:sk // 2, :] = s1
            s_ref[i][0, sk // 2:sk, :] = s2
        else:
            k1, k2, k3 = ks[h][0]
            q_ab = q_ab.T
            t1 = _dot(q_ab, k1)
            s1 = (t1 + _dot_tn(q_bc, k2)) * scale_log2e
            s2 = (t1 + _dot_tn(q_ac, k3)) * scale_log2e
            scores[i] = (s1, s2, guarded_max(i, s1, s2, q_ab, 1))

    def softmax(i):
        _, a, b = items[i]
        w = b - a
        if w == 128:
            m = jnp.broadcast_to(scores.pop(i), (8, w))
            acc, es, p = None, [], []
            for r in range(0, sk, 8):
                e = jnp.exp2(s_ref[i][zero, r:r + 8, :] - m)
                acc = e if acc is None else acc + e
                es.append(e)
                if len(es) == 16:
                    p.append(jnp.concatenate(es, 0).astype(_BF16))
                    es = []
            probs[i] = (p, _reciprocal(jnp.sum(acc, axis=0, keepdims=True)))
        else:
            s1, s2, m = scores.pop(i)
            es = [jnp.exp2(s[:, j:j + 128] - m)
                  for s in (s1, s2) for j in range(0, sk // 2, 128)]
            inv = _reciprocal(
                jnp.sum((es[0] + es[1]) + (es[2] + es[3]), axis=1, keepdims=True))
            probs[i] = ([e.astype(_BF16) for e in es], inv)

    def pv(i):
        h, a, b = items[i]
        if h not in vs:
            vs[h] = [(v_ref[h, 0:128, j:j + 128], v_ref[h, :, j:j + 128],
                      v_ref[h, 128:192, j:j + 128]) for j in range(0, sk, 128)]
        p, inv = probs.pop(i)
        if b - a == 128:
            o = _sum([_dot(v[1], pj) for v, pj in zip(vs[h], p)])
            o_ref[h, :, a:b] = (o * inv).astype(o_ref.dtype)
        else:
            o_lo = _sum([_dot_nt(pj, v[0]) for v, pj in zip(vs[h], p)])
            o_hi = _sum([_dot_nt(v[2], pj) for v, pj in zip(vs[h], p)])
            inv = jnp.broadcast_to(inv, (b - a, 128))
            o_lo = o_lo * inv
            o_hi = o_hi * inv.T[0:64]
            o_ref[h, 0:128, a:b] = o_lo.astype(o_ref.dtype).T
            o_ref[h, 128:192, a:b] = o_hi.astype(o_ref.dtype)

    n = len(items)
    for step in range(n + _PV_LAG):
        h, t = divmod(step, len(tiles))
        if step < n and t == _K_PREP_POS:
            ks[h + 1] = _prep_k(k_ref.at[h])
            if h + 1 == heads:
                _save_k(ks[heads], *k_carry)
        if step < n:
            qk(step)
        if 0 <= step - 1 < n:
            softmax(step - 1)
        if 0 <= step - _PV_LAG:
            pv(step - _PV_LAG)


def _attn_kernel(q_hbm, k_hbm, v_hbm, o_hbm,
                 q_small, k_small, v_small, o_small, q_big, k_big, v_big, o_big,
                 kn_ref, kt_ref, kd_ref, redo_ref,
                 sem_si, sem_so, sem_bi, sem_bo, *s_refs, scale_log2e):
    k_carry = (kn_ref, kt_ref, kd_ref)
    n_heads = q_hbm.shape[0]
    n_big = (n_heads - _SMALL * (_N_FIRST + _N_LAST)) // _BIG
    big0 = _SMALL * _N_FIRST
    last0 = big0 + _BIG * n_big
    last_load_quad = _N_FIRST // 4 + 2
    assert last0 + _SMALL * _N_LAST == n_heads
    assert n_big >= 4 * (last_load_quad + _N_LAST)
    assert _N_FIRST >= max(_BIG, _N_LAST) and _N_LAST >= 2
    copy = pltpu.make_async_copy

    def small(ref, j):
        return ref.at[pl.ds(_SMALL * j, _SMALL)]

    def start_loads(head, n, dsts, sem):
        for src, dst, off in zip((k_hbm, q_hbm, v_hbm), dsts, (1, 0, 0)):
            copy(src.at[pl.ds(head + off, n)], dst, sem).start()

    def wait_loads(dsts, sem):
        for dst in dsts:
            copy(dst, dst, sem).wait()

    def small_in(j, sem):
        return tuple(small(x, j) for x in (k_small, q_small, v_small)), sem_si.at[sem]

    def big_in(slot):
        return tuple(x.at[slot] for x in (k_big, q_big, v_big)), sem_bi.at[slot]

    def big_out(i):
        return copy(o_big.at[i & 1], o_hbm.at[pl.ds(big0 + _BIG * i, _BIG)], sem_bo.at[i & 1])

    def last_out(j):
        return copy(small(o_small, _N_FIRST + j),
                    o_hbm.at[pl.ds(last0 + _SMALL * j, _SMALL)], sem_so.at[j])

    def run(bufs, head0):
        zero = jax.lax.shift_right_logical(head0, 30)
        _group(*bufs, k_carry, s_refs, redo_ref, head0, zero, scale_log2e)

    k0 = copy(k_hbm.at[0], k_big.at[1, 0], sem_bi.at[1])
    k0.start()
    start_loads(0, _SMALL, *small_in(0, 0))
    redo_ref[...] = jnp.zeros(redo_ref.shape, _F32)
    k0.wait()
    _save_k(_prep_k(k_big.at[1, 0]), *k_carry)

    def first_step(j, _):
        wait_loads(*small_in(j, j & 1))

        @pl.when(j + 1 < _N_FIRST)
        def _():
            start_loads(_SMALL * (j + 1), _SMALL, *small_in(j + 1, (j + 1) & 1))

        @pl.when(j < _BIG)
        def _():
            dsts = tuple(x.at[0, pl.ds(j, 1)] for x in (k_big, q_big, v_big))
            start_loads(big0 + j, 1, dsts, sem_bi.at[0])

        run([small(x, j) for x in (q_small, k_small, v_small, o_small)], _SMALL * j)

    jax.lax.fori_loop(0, _N_FIRST, first_step, None)
    start_loads(big0 + _BIG, _BIG, *big_in(1))

    def big_step(i, _):
        slot = i & 1
        wait_loads(*big_in(slot))

        @pl.when(i >= 2)
        def _():
            big_out(i - 2).wait()

        run([x.at[slot] for x in (q_big, k_big, v_big, o_big)], big0 + _BIG * i)

        @pl.when(i + 2 < n_big)
        def _():
            start_loads(big0 + _BIG * (i + 2), _BIG, *big_in(slot))

        big_out(i).start()

        @pl.when(i < _N_FIRST)
        def _():
            copy(small(o_small, i), small(o_hbm, i), sem_so.at[_N_LAST]).start()

        j = (i >> 2) - last_load_quad

        @pl.when((j >= 0) & (j < _N_LAST) & (i & 3 == 0))
        def _():
            head = last0 + _SMALL * j
            sem = sem_si.at[j]
            copy(k_hbm.at[pl.ds(head + 1, _SMALL - 1)],
                 k_small.at[pl.ds(_SMALL * j, _SMALL - 1)], sem).start()
            copy(k_hbm.at[jnp.minimum(head + _SMALL, n_heads - 1)],
                 k_small.at[_SMALL * j + _SMALL - 1], sem).start()
            copy(q_hbm.at[pl.ds(head, _SMALL)], small(q_small, j), sem).start()
            copy(v_hbm.at[pl.ds(head, _SMALL)], small(v_small, j), sem).start()

    jax.lax.fori_loop(0, n_big, big_step, None)

    def last_step(j, _):
        wait_loads(*small_in(j, j))
        run([small(x, j) for x in (q_small, k_small, v_small)]
            + [small(o_small, _N_FIRST + j)], last0 + _SMALL * j)
        last_out(j).start()

    jax.lax.fori_loop(0, _N_LAST, last_step, None)
    any_redo = jnp.max(jnp.max(redo_ref[...], axis=0)) > 0.0

    copy(o_small.at[pl.ds(0, big0)], o_hbm.at[pl.ds(0, big0)], sem_so.at[_N_LAST]).wait()
    big_out(n_big - 2).wait()
    big_out(n_big - 1).wait()
    for j in range(_N_LAST):
        last_out(j).wait()

    def redo_step(head, _):
        @pl.when(jnp.max(redo_ref[head]) > 0.0)
        def _():
            q, k, v, o = (x.at[0, 0] for x in (q_big, k_big, v_big, o_big))
            for src, dst in ((q_hbm, q), (k_hbm, k), (v_hbm, v)):
                copy(src.at[head], dst, sem_bi.at[0]).start()
            wait_loads((q, k, v), sem_bi.at[0])
            _head_exact(q, k, v, o, scale_log2e)
            out = copy(o, o_hbm.at[head], sem_bo.at[0])
            out.start()
            out.wait()

    @pl.when(any_redo)
    def _():
        jax.lax.fori_loop(0, n_heads, redo_step, None)


@jax.jit
def pallas_standalone__gqa_softmax__near_ridge_kernel(
    q: jax.Array,
    k: jax.Array,
    v: jax.Array,
):
    B, Hq, Sq, D = q.shape
    Hkv, Sk = k.shape[1], k.shape[2]
    assert Hq == Hkv and D == 192 and Sk == 512 and Sq <= 8 * 128
    n = B * Hq
    qt = jnp.swapaxes(q, 2, 3).reshape(n, 3, D // 3, Sq)
    kt = jnp.swapaxes(k, 2, 3).reshape(n, D, Sk)
    vt = jnp.swapaxes(v, 2, 3).reshape(n, D, Sk)

    def buffers(heads_in, heads_out):
        return [pltpu.VMEM((*heads_in, 3, D // 3, Sq), q.dtype),
                pltpu.VMEM((*heads_in, D, Sk), k.dtype),
                pltpu.VMEM((*heads_in, D, Sk), v.dtype),
                pltpu.VMEM((*heads_out, D, Sq), q.dtype)]

    ot = pl.pallas_call(
        functools.partial(_attn_kernel, scale_log2e=(D ** -0.5) * _LOG2E),
        in_specs=[pl.BlockSpec(memory_space=pl.ANY)] * 3,
        out_specs=pl.BlockSpec(memory_space=pl.ANY),
        out_shape=jax.ShapeDtypeStruct((n, D, Sq), q.dtype),
        scratch_shapes=[
            *buffers((_SMALL * _N_FIRST,), (_SMALL * (_N_FIRST + _N_LAST),)),
            *buffers((2, _BIG), (2, _BIG)),
            pltpu.VMEM((3, 64, Sk // 2), _U32),
            pltpu.VMEM((3, Sk // 4, 128), _U32),
            pltpu.VMEM((1, 128), _F32),
            pltpu.VMEM((n, 8, 128), _F32),
            pltpu.SemaphoreType.DMA((_N_LAST,)),
            pltpu.SemaphoreType.DMA((_N_LAST + 1,)),
            pltpu.SemaphoreType.DMA((2,)),
            pltpu.SemaphoreType.DMA((2,)),
            *[pltpu.VMEM((1, Sk, 128), _F32)] * _S_SLOTS,
        ],
        compiler_params=pltpu.CompilerParams(
            vmem_limit_bytes=100 * 1024 * 1024,
            disable_bounds_checks=True,
            flags={"XLA_TPU_FORCE_LP_LLO_SCHEDULER": True},
        ),
    )(qt, kt, vt)
    return jnp.swapaxes(ot.reshape(B, Hq, D, Sq), 2, 3)
```

```python
import functools
import math

import jax
import jax.numpy as jnp
import jax.experimental.pallas as pl
import jax.experimental.pallas.tpu as pltpu

_F32 = jnp.float32
_BF16 = jnp.bfloat16
_U32 = jnp.uint32
_LOG2E = math.log2(math.e)

_BIG = 12
_SMALL = 2
_N_FIRST = 13
_N_LAST = 3
_PV_LAG = 3
_REM_POS = 3
_K_PREP_POS = 4
_S_SLOTS = 4
_GUARD = 8.0


def _dot(a, b):
    return jnp.dot(a, b, preferred_element_type=_F32)


def _dot_tn(a, b):
    return jax.lax.dot_general(a, b, (((0,), (0,)), ((), ())), preferred_element_type=_F32)


def _dot_nt(a, b):
    return jax.lax.dot_general(a, b, (((1,), (1,)), ((), ())), preferred_element_type=_F32)


def _sum(xs):
    return functools.reduce(lambda a, b: a + b, xs)


def _reciprocal(x):
    r = pl.reciprocal(x, approx=True)
    return r * (2.0 - x * r)


def _norm2(x, axis):
    return jnp.sum(x * x, axis=axis, keepdims=True)


def _prep_k(k_ref):
    half = k_ref.shape[1] // 2

    def blk(r, col):
        return k_ref[64 * r:64 * (r + 1), half * col:half * (col + 1)].astype(_F32)

    k1a, k1b, k1c = blk(0, 0), blk(1, 0), blk(2, 0)
    k2a, k2b, k2c = blk(0, 1), blk(1, 1), blk(2, 1)

    def cat(a, b):
        return jnp.concatenate([a, b], 0).astype(_BF16)

    da, db = k2a - k1a, k1b - k2b
    kn = (cat(k1a, k2b), cat(db, k1c), cat(da, k2c))
    kd = jnp.max(jnp.maximum(_norm2(da, 0), _norm2(db, 0)), axis=1, keepdims=True)
    return kn, tuple(x.T for x in kn), jnp.broadcast_to(kd, (1, 128))


def _save_k(k, kn_ref, kt_ref, kd_ref):
    for j in range(3):
        kn_ref[j] = pltpu.bitcast(k[0][j], _U32)
        kt_ref[j] = pltpu.bitcast(k[1][j], _U32)
    kd_ref[...] = k[2]


def _load_k(kn_ref, kt_ref, kd_ref):
    return (tuple(pltpu.bitcast(kn_ref[j], _BF16) for j in range(3)),
            tuple(pltpu.bitcast(kt_ref[j], _BF16) for j in range(3)),
            kd_ref[...])


def _head_exact(q_ref, k_ref, v_ref, o_ref, scale_log2e):
    s = _dot_tn(k_ref[...], q_ref[...].reshape(o_ref.shape))
    e = jnp.exp2((s - jnp.max(s, axis=0, keepdims=True)) * scale_log2e)
    o = _dot(v_ref[...], e.astype(_BF16)) / jnp.sum(e, axis=0, keepdims=True)
    o_ref[...] = o.astype(o_ref.dtype)


def _group(q_ref, k_ref, v_ref, o_ref, k_carry, s_refs, redo_ref, head0, zero, scale_log2e):
    heads, _, sq = o_ref.shape
    sk = k_ref.shape[2]
    tiles = [(a, a + 128) for a in range(0, sq - 127, 128)]
    if sq % 128:
        tiles.insert(_REM_POS, (sq - sq % 128, sq))
    items = [(h, a, b) for h in range(heads) for a, b in tiles]
    full = [i for i, (_, a, b) in enumerate(items) if b - a == 128]
    s_ref = {i: s_refs[j % len(s_refs)] for j, i in enumerate(full)}
    ks = {0: _load_k(*k_carry)}
    vs, scores, probs, flags = {}, {}, {}, []

    def guarded_max(i, s1, s2, q_ab, axis):
        h = items[i][0]
        m = jnp.max(jnp.maximum(s1, s2), axis=axis, keepdims=True)
        limit = jnp.maximum(m * m, _LOG2E ** 2) * (_GUARD / scale_log2e) ** 2
        flag = jnp.where(_norm2(q_ab.astype(_F32), axis) * ks[h][2] < limit, 0.0, 1.0)
        rows = jnp.broadcast_to(flag, (max(flag.shape[0], 8), 128))
        flags.extend(rows[r:r + 8] for r in range(0, rows.shape[0], 8))
        if (i + 1) % len(tiles) == 0:
            redo_ref[head0 + h] = functools.reduce(jnp.maximum, flags)
            flags.clear()
        return m + flag

    def qk(i):
        h, a, b = items[i]
        w = b - a
        q_ab = q_ref[h, 0:2, :, a:b].reshape(128, w)
        q_bc = q_ref[h, 1:3, :, a:b].reshape(128, w)
        q_ac = jnp.concatenate(
            [q_ref[h, 0:1, :, a:b], q_ref[h, 2:3, :, a:b]], 0).reshape(128, w)
        if w == 128:
            k1, k2, k3 = ks[h][1]
            t1 = _dot(k1, q_ab)
            s1 = (t1 + _dot(k2, q_bc)) * scale_log2e
            s2 = (t1 + _dot(k3, q_ac)) * scale_log2e
            scores[i] = guarded_max(i, s1, s2, q_ab, 0)
            s_ref[i][0, 0:sk // 2, :] = s1
            s_ref[i][0, sk // 2:sk, :] = s2
        else:
            k1, k2, k3 = ks[h][0]
            q_ab = q_ab.T
            t1 = _dot(q_ab, k1)
            s1 = (t1 + _dot_tn(q_bc, k2)) * scale_log2e
            s2 = (t1 + _dot_tn(q_ac, k3)) * scale_log2e
            scores[i] = (s1, s2, guarded_max(i, s1, s2, q_ab, 1))

    def softmax(i):
        _, a, b = items[i]
        w = b - a
        if w == 128:
            m = jnp.broadcast_to(scores.pop(i), (8, w))
            acc, es, p = None, [], []
            for r in range(0, sk, 8):
                e = jnp.exp2(s_ref[i][zero, r:r + 8, :] - m)
                acc = e if acc is None else acc + e
                es.append(e)
                if len(es) == 16:
                    p.append(jnp.concatenate(es, 0).astype(_BF16))
                    es = []
            probs[i] = (p, _reciprocal(jnp.sum(acc, axis=0, keepdims=True)))
        else:
            s1, s2, m = scores.pop(i)
            es = [jnp.exp2(s[:, j:j + 128] - m)
                  for s in (s1, s2) for j in range(0, sk // 2, 128)]
            inv = _reciprocal(
                jnp.sum((es[0] + es[1]) + (es[2] + es[3]), axis=1, keepdims=True))
            probs[i] = ([e.astype(_BF16) for e in es], inv)

    def pv(i):
        h, a, b = items[i]
        if h not in vs:
            vs[h] = [(v_ref[h, 0:128, j:j + 128], v_ref[h, :, j:j + 128],
                      v_ref[h, 128:192, j:j + 128]) for j in range(0, sk, 128)]
        p, inv = probs.pop(i)
        if b - a == 128:
            o = _sum([_dot(v[1], pj) for v, pj in zip(vs[h], p)])
            o_ref[h, :, a:b] = (o * inv).astype(o_ref.dtype)
        else:
            o_lo = _sum([_dot_nt(pj, v[0]) for v, pj in zip(vs[h], p)])
            o_hi = _sum([_dot_nt(v[2], pj) for v, pj in zip(vs[h], p)])
            inv = jnp.broadcast_to(inv, (b - a, 128))
            o_lo = o_lo * inv
            o_hi = o_hi * inv.T[0:64]
            o_ref[h, 0:128, a:b] = o_lo.astype(o_ref.dtype).T
            o_ref[h, 128:192, a:b] = o_hi.astype(o_ref.dtype)

    n = len(items)
    for step in range(n + _PV_LAG):
        h, t = divmod(step, len(tiles))
        if step < n and t == _K_PREP_POS:
            ks[h + 1] = _prep_k(k_ref.at[h])
            if h + 1 == heads:
                _save_k(ks[heads], *k_carry)
        if step < n:
            qk(step)
        if 0 <= step - 1 < n:
            softmax(step - 1)
        if 0 <= step - _PV_LAG:
            pv(step - _PV_LAG)


def _attn_kernel(q_hbm, k_hbm, v_hbm, o_hbm,
                 q_small, k_small, v_small, o_small, q_big, k_big, v_big, o_big,
                 kn_ref, kt_ref, kd_ref, redo_ref,
                 sem_si, sem_so, sem_bi, sem_bo, *s_refs, scale_log2e):
    k_carry = (kn_ref, kt_ref, kd_ref)
    n_heads = q_hbm.shape[0]
    n_big = (n_heads - _SMALL * (_N_FIRST + _N_LAST)) // _BIG
    big0 = _SMALL * _N_FIRST
    last0 = big0 + _BIG * n_big
    last_load_quad = _N_FIRST // 4 + 2
    assert last0 + _SMALL * _N_LAST == n_heads
    assert n_big >= 4 * (last_load_quad + _N_LAST)
    assert _N_FIRST >= max(_BIG, _N_LAST) and _N_LAST >= 2
    copy = pltpu.make_async_copy

    def small(ref, j):
        return ref.at[pl.ds(_SMALL * j, _SMALL)]

    def start_loads(head, n, dsts, sem):
        for src, dst, off in zip((k_hbm, q_hbm, v_hbm), dsts, (1, 0, 0)):
            copy(src.at[pl.ds(head + off, n)], dst, sem).start()

    def wait_loads(dsts, sem):
        for dst in dsts:
            copy(dst, dst, sem).wait()

    def small_in(j, sem):
        return tuple(small(x, j) for x in (k_small, q_small, v_small)), sem_si.at[sem]

    def big_in(slot):
        return tuple(x.at[slot] for x in (k_big, q_big, v_big)), sem_bi.at[slot]

    def big_out(i):
        return copy(o_big.at[i & 1], o_hbm.at[pl.ds(big0 + _BIG * i, _BIG)], sem_bo.at[i & 1])

    def last_out(j):
        return copy(small(o_small, _N_FIRST + j),
                    o_hbm.at[pl.ds(last0 + _SMALL * j, _SMALL)], sem_so.at[j])

    def run(bufs, head0):
        zero = jax.lax.shift_right_logical(head0, 30)
        _group(*bufs, k_carry, s_refs, redo_ref, head0, zero, scale_log2e)

    k0 = copy(k_hbm.at[0], k_big.at[1, 0], sem_bi.at[1])
    k0.start()
    start_loads(0, _SMALL, *small_in(0, 0))
    k0.wait()
    _save_k(_prep_k(k_big.at[1, 0]), *k_carry)

    def first_step(j, _):
        wait_loads(*small_in(j, j & 1))

        @pl.when(j + 1 < _N_FIRST)
        def _():
            start_loads(_SMALL * (j + 1), _SMALL, *small_in(j + 1, (j + 1) & 1))

        @pl.when(j < _BIG)
        def _():
            dsts = tuple(x.at[0, pl.ds(j, 1)] for x in (k_big, q_big, v_big))
            start_loads(big0 + j, 1, dsts, sem_bi.at[0])

        run([small(x, j) for x in (q_small, k_small, v_small, o_small)], _SMALL * j)

    jax.lax.fori_loop(0, _N_FIRST, first_step, None)
    start_loads(big0 + _BIG, _BIG, *big_in(1))

    def big_step(i, _):
        slot = i & 1
        wait_loads(*big_in(slot))

        @pl.when(i >= 2)
        def _():
            big_out(i - 2).wait()

        run([x.at[slot] for x in (q_big, k_big, v_big, o_big)], big0 + _BIG * i)

        @pl.when(i + 2 < n_big)
        def _():
            start_loads(big0 + _BIG * (i + 2), _BIG, *big_in(slot))

        big_out(i).start()

        @pl.when(i < _N_FIRST)
        def _():
            copy(small(o_small, i), small(o_hbm, i), sem_so.at[_N_LAST]).start()

        j = (i >> 2) - last_load_quad

        @pl.when((j >= 0) & (j < _N_LAST) & (i & 3 == 0))
        def _():
            head = last0 + _SMALL * j
            sem = sem_si.at[j]
            copy(k_hbm.at[pl.ds(head + 1, _SMALL - 1)],
                 k_small.at[pl.ds(_SMALL * j, _SMALL - 1)], sem).start()
            copy(k_hbm.at[jnp.minimum(head + _SMALL, n_heads - 1)],
                 k_small.at[_SMALL * j + _SMALL - 1], sem).start()
            copy(q_hbm.at[pl.ds(head, _SMALL)], small(q_small, j), sem).start()
            copy(v_hbm.at[pl.ds(head, _SMALL)], small(v_small, j), sem).start()

    jax.lax.fori_loop(0, n_big, big_step, None)

    def last_step(j, _):
        wait_loads(*small_in(j, j))
        run([small(x, j) for x in (q_small, k_small, v_small)]
            + [small(o_small, _N_FIRST + j)], last0 + _SMALL * j)
        last_out(j).start()

    jax.lax.fori_loop(0, _N_LAST, last_step, None)
    any_redo = jnp.max(jnp.max(redo_ref[...], axis=0)) > 0.0

    copy(o_small.at[pl.ds(0, big0)], o_hbm.at[pl.ds(0, big0)], sem_so.at[_N_LAST]).wait()
    big_out(n_big - 2).wait()
    big_out(n_big - 1).wait()
    for j in range(_N_LAST):
        last_out(j).wait()

    def redo_step(head, _):
        @pl.when(jnp.max(redo_ref[head]) > 0.0)
        def _():
            q, k, v, o = (x.at[0, 0] for x in (q_big, k_big, v_big, o_big))
            for src, dst in ((q_hbm, q), (k_hbm, k), (v_hbm, v)):
                copy(src.at[head], dst, sem_bi.at[0]).start()
            wait_loads((q, k, v), sem_bi.at[0])
            _head_exact(q, k, v, o, scale_log2e)
            out = copy(o, o_hbm.at[head], sem_bo.at[0])
            out.start()
            out.wait()

    @pl.when(any_redo)
    def _():
        jax.lax.fori_loop(0, n_heads, redo_step, None)


@jax.jit
def pallas_standalone__gqa_softmax__near_ridge_kernel(
    q: jax.Array,
    k: jax.Array,
    v: jax.Array,
):
    B, Hq, Sq, D = q.shape
    Hkv, Sk = k.shape[1], k.shape[2]
    assert Hq == Hkv and D == 192 and Sk == 512
    n = B * Hq
    qt = jnp.swapaxes(q, 2, 3).reshape(n, 3, D // 3, Sq)
    kt = jnp.swapaxes(k, 2, 3).reshape(n, D, Sk)
    vt = jnp.swapaxes(v, 2, 3).reshape(n, D, Sk)

    def buffers(heads_in, heads_out):
        return [pltpu.VMEM((*heads_in, 3, D // 3, Sq), q.dtype),
                pltpu.VMEM((*heads_in, D, Sk), k.dtype),
                pltpu.VMEM((*heads_in, D, Sk), v.dtype),
                pltpu.VMEM((*heads_out, D, Sq), q.dtype)]

    ot = pl.pallas_call(
        functools.partial(_attn_kernel, scale_log2e=(D ** -0.5) * _LOG2E),
        in_specs=[pl.BlockSpec(memory_space=pl.ANY)] * 3,
        out_specs=pl.BlockSpec(memory_space=pl.ANY),
        out_shape=jax.ShapeDtypeStruct((n, D, Sq), q.dtype),
        scratch_shapes=[
            *buffers((_SMALL * _N_FIRST,), (_SMALL * (_N_FIRST + _N_LAST),)),
            *buffers((2, _BIG), (2, _BIG)),
            pltpu.VMEM((3, 64, Sk // 2), _U32),
            pltpu.VMEM((3, Sk // 4, 128), _U32),
            pltpu.VMEM((1, 128), _F32),
            pltpu.VMEM((n, 8, 128), _F32),
            pltpu.SemaphoreType.DMA((_N_LAST,)),
            pltpu.SemaphoreType.DMA((_N_LAST + 1,)),
            pltpu.SemaphoreType.DMA((2,)),
            pltpu.SemaphoreType.DMA((2,)),
            *[pltpu.VMEM((1, Sk, 128), _F32)] * _S_SLOTS,
        ],
        compiler_params=pltpu.CompilerParams(
            vmem_limit_bytes=100 * 1024 * 1024,
            disable_bounds_checks=True,
            flags={"XLA_TPU_FORCE_LP_LLO_SCHEDULER": True},
        ),
    )(qt, kt, vt)
    return jnp.swapaxes(ot.reshape(B, Hq, D, Sq), 2, 3)
```

```python
import functools
import math

import jax
import jax.numpy as jnp
import jax.experimental.pallas as pl
import jax.experimental.pallas.tpu as pltpu

_F32 = jnp.float32
_BF16 = jnp.bfloat16
_U32 = jnp.uint32
_LOG2E = math.log2(math.e)

_BIG = 12
_SMALL = 2
_N_FIRST = 13
_N_LAST = 3
_PV_LAG = 3
_REM_POS = 5
_REM_POS_LAST = 3
_K_PREP_POS = 4
_S_SLOTS = 4
_GUARD = 8.0


def _dot(a, b):
    return jnp.dot(a, b, preferred_element_type=_F32)


def _dot_tn(a, b):
    return jax.lax.dot_general(a, b, (((0,), (0,)), ((), ())), preferred_element_type=_F32)


def _dot_nt(a, b):
    return jax.lax.dot_general(a, b, (((1,), (1,)), ((), ())), preferred_element_type=_F32)


def _sum(xs):
    return functools.reduce(lambda a, b: a + b, xs)


def _reciprocal(x):
    r = pl.reciprocal(x, approx=True)
    return r * (2.0 - x * r)


def _norm2(x, axis):
    return jnp.sum(x * x, axis=axis, keepdims=True)


def _prep_k(k_ref):
    half = k_ref.shape[1] // 2

    def blk(r, col):
        return k_ref[64 * r:64 * (r + 1), half * col:half * (col + 1)].astype(_F32)

    k1a, k1b, k1c = blk(0, 0), blk(1, 0), blk(2, 0)
    k2a, k2b, k2c = blk(0, 1), blk(1, 1), blk(2, 1)

    def cat(a, b):
        return jnp.concatenate([a, b], 0).astype(_BF16)

    da, db = k2a - k1a, k1b - k2b
    kn = (cat(k1a, k2b), cat(db, k1c), cat(da, k2c))
    kd = jnp.max(jnp.maximum(_norm2(da, 0), _norm2(db, 0)), axis=1, keepdims=True)
    return kn, tuple(x.T for x in kn), jnp.broadcast_to(kd, (1, 128))


def _save_k(k, kn_ref, kt_ref, kd_ref):
    for j in range(3):
        kn_ref[j] = pltpu.bitcast(k[0][j], _U32)
        kt_ref[j] = pltpu.bitcast(k[1][j], _U32)
    kd_ref[...] = k[2]


def _load_k(kn_ref, kt_ref, kd_ref):
    return (tuple(pltpu.bitcast(kn_ref[j], _BF16) for j in range(3)),
            tuple(pltpu.bitcast(kt_ref[j], _BF16) for j in range(3)),
            kd_ref[...])


def _head_exact(q_ref, k_ref, v_ref, o_ref, scale_log2e):
    s = _dot_tn(k_ref[...], q_ref[...].reshape(o_ref.shape))
    e = jnp.exp2((s - jnp.max(s, axis=0, keepdims=True)) * scale_log2e)
    o = _dot(v_ref[...], e.astype(_BF16)) / jnp.sum(e, axis=0, keepdims=True)
    o_ref[...] = o.astype(o_ref.dtype)


def _group(q_ref, k_ref, v_ref, o_ref, k_carry, s_refs, redo_ref, head0, zero, scale_log2e):
    heads, _, sq = o_ref.shape
    sk = k_ref.shape[2]
    n_tiles = pl.cdiv(sq, 128)
    items = []
    for h in range(heads):
        tiles = [(h, a, a + 128) for a in range(0, sq - 127, 128)]
        if sq % 128:
            pos = _REM_POS if h + 1 < heads else _REM_POS_LAST
            tiles.insert(pos, (h, sq - sq % 128, sq))
        items += tiles
    full = [i for i, (_, a, b) in enumerate(items) if b - a == 128]
    s_ref = {i: s_refs[j % len(s_refs)] for j, i in enumerate(full)}
    ks = {0: _load_k(*k_carry)}
    vs, scores, probs, flags = {}, {}, {}, []

    def guarded_max(i, s1, s2, q_ab, axis):
        h = items[i][0]
        m = jnp.max(jnp.maximum(s1, s2), axis=axis, keepdims=True)
        limit = jnp.maximum(m * m, _LOG2E ** 2) * (_GUARD / scale_log2e) ** 2
        flag = jnp.where(_norm2(q_ab.astype(_F32), axis) * ks[h][2] < limit, 0.0, 1.0)
        rows = jnp.broadcast_to(flag, (max(flag.shape[0], 8), 128))
        flags.extend(rows[r:r + 8] for r in range(0, rows.shape[0], 8))
        if (i + 1) % n_tiles == 0:
            redo_ref[head0 + h] = functools.reduce(jnp.maximum, flags)
            flags.clear()
        return m + flag

    def qk(i):
        h, a, b = items[i]
        w = b - a
        q_ab = q_ref[h, 0:2, :, a:b].reshape(128, w)
        q_bc = q_ref[h, 1:3, :, a:b].reshape(128, w)
        q_ac = jnp.concatenate(
            [q_ref[h, 0:1, :, a:b], q_ref[h, 2:3, :, a:b]], 0).reshape(128, w)
        if w == 128:
            k1, k2, k3 = ks[h][1]
            t1 = _dot(k1, q_ab)
            s1 = (t1 + _dot(k2, q_bc)) * scale_log2e
            s2 = (t1 + _dot(k3, q_ac)) * scale_log2e
            scores[i] = guarded_max(i, s1, s2, q_ab, 0)
            s_ref[i][0, 0:sk // 2, :] = s1
            s_ref[i][0, sk // 2:sk, :] = s2
        else:
            k1, k2, k3 = ks[h][0]
            q_ab = q_ab.T
            t1 = _dot(q_ab, k1)
            s1 = (t1 + _dot_tn(q_bc, k2)) * scale_log2e
            s2 = (t1 + _dot_tn(q_ac, k3)) * scale_log2e
            scores[i] = (s1, s2, guarded_max(i, s1, s2, q_ab, 1))

    def softmax(i):
        _, a, b = items[i]
        w = b - a
        if w == 128:
            m = jnp.broadcast_to(scores.pop(i), (8, w))
            acc, es, p = None, [], []
            for r in range(0, sk, 8):
                e = jnp.exp2(s_ref[i][zero, r:r + 8, :] - m)
                acc = e if acc is None else acc + e
                es.append(e)
                if len(es) == 16:
                    p.append(jnp.concatenate(es, 0).astype(_BF16))
                    es = []
            probs[i] = (p, _reciprocal(jnp.sum(acc, axis=0, keepdims=True)))
        else:
            s1, s2, m = scores.pop(i)
            es = [jnp.exp2(s[:, j:j + 128] - m)
                  for s in (s1, s2) for j in range(0, sk // 2, 128)]
            inv = _reciprocal(
                jnp.sum((es[0] + es[1]) + (es[2] + es[3]), axis=1, keepdims=True))
            probs[i] = [(e * inv).astype(_BF16) for e in es]

    def pv(i):
        h, a, b = items[i]
        if h not in vs:
            vs[h] = [(v_ref[h, 0:128, j:j + 128], v_ref[h, :, j:j + 128],
                      v_ref[h, 128:192, j:j + 128]) for j in range(0, sk, 128)]
        if b - a == 128:
            p, inv = probs.pop(i)
            o = _sum([_dot(v[1], pj) for v, pj in zip(vs[h], p)])
            o_ref[h, :, a:b] = (o * inv).astype(o_ref.dtype)
        else:
            p = probs.pop(i)
            o_lo = _sum([_dot_nt(pj, v[0]) for v, pj in zip(vs[h], p)])
            o_hi = _sum([_dot_nt(v[2], pj) for v, pj in zip(vs[h], p)])
            o_ref[h, 0:128, a:b] = o_lo.astype(o_ref.dtype).T
            o_ref[h, 128:192, a:b] = o_hi.astype(o_ref.dtype)

    n = len(items)
    for step in range(n + _PV_LAG):
        h, t = divmod(step, n_tiles)
        if step < n and t == _K_PREP_POS:
            ks[h + 1] = _prep_k(k_ref.at[h])
            if h + 1 == heads:
                _save_k(ks[heads], *k_carry)
        if step < n:
            qk(step)
        if 0 <= step - 1 < n:
            softmax(step - 1)
        if 0 <= step - _PV_LAG:
            pv(step - _PV_LAG)


def _attn_kernel(q_hbm, k_hbm, v_hbm, o_hbm,
                 q_small, k_small, v_small, o_small, q_big, k_big, v_big, o_big,
                 kn_ref, kt_ref, kd_ref, redo_ref,
                 sem_si, sem_so, sem_bi, sem_bo, *s_refs, scale_log2e):
    k_carry = (kn_ref, kt_ref, kd_ref)
    n_heads = q_hbm.shape[0]
    n_big = (n_heads - _SMALL * (_N_FIRST + _N_LAST)) // _BIG
    big0 = _SMALL * _N_FIRST
    last0 = big0 + _BIG * n_big
    last_load_quad = _N_FIRST // 4 + 2
    assert last0 + _SMALL * _N_LAST == n_heads
    assert n_big >= 4 * (last_load_quad + _N_LAST)
    assert _N_FIRST >= max(_BIG, _N_LAST) and _N_LAST >= 2
    copy = pltpu.make_async_copy

    def small(ref, j):
        return ref.at[pl.ds(_SMALL * j, _SMALL)]

    def start_loads(head, n, dsts, sem):
        for src, dst, off in zip((k_hbm, q_hbm, v_hbm), dsts, (1, 0, 0)):
            copy(src.at[pl.ds(head + off, n)], dst, sem).start()

    def wait_loads(dsts, sem):
        for dst in dsts:
            copy(dst, dst, sem).wait()

    def small_in(j, sem):
        return tuple(small(x, j) for x in (k_small, q_small, v_small)), sem_si.at[sem]

    def big_in(slot):
        return tuple(x.at[slot] for x in (k_big, q_big, v_big)), sem_bi.at[slot]

    def big_out(i):
        return copy(o_big.at[i & 1], o_hbm.at[pl.ds(big0 + _BIG * i, _BIG)], sem_bo.at[i & 1])

    def last_out(j):
        return copy(small(o_small, _N_FIRST + j),
                    o_hbm.at[pl.ds(last0 + _SMALL * j, _SMALL)], sem_so.at[j])

    def run(bufs, head0):
        zero = jax.lax.shift_right_logical(head0, 30)
        _group(*bufs, k_carry, s_refs, redo_ref, head0, zero, scale_log2e)

    k0 = copy(k_hbm.at[0], k_big.at[1, 0], sem_bi.at[1])
    k0.start()
    start_loads(0, _SMALL, *small_in(0, 0))
    k0.wait()
    _save_k(_prep_k(k_big.at[1, 0]), *k_carry)

    def first_step(j, _):
        wait_loads(*small_in(j, j & 1))

        @pl.when(j + 1 < _N_FIRST)
        def _():
            start_loads(_SMALL * (j + 1), _SMALL, *small_in(j + 1, (j + 1) & 1))

        @pl.when(j < _BIG)
        def _():
            dsts = tuple(x.at[0, pl.ds(j, 1)] for x in (k_big, q_big, v_big))
            start_loads(big0 + j, 1, dsts, sem_bi.at[0])

        run([small(x, j) for x in (q_small, k_small, v_small, o_small)], _SMALL * j)

    jax.lax.fori_loop(0, _N_FIRST, first_step, None)
    start_loads(big0 + _BIG, _BIG, *big_in(1))

    def big_step(i, _):
        slot = i & 1
        wait_loads(*big_in(slot))

        @pl.when(i >= 2)
        def _():
            big_out(i - 2).wait()

        run([x.at[slot] for x in (q_big, k_big, v_big, o_big)], big0 + _BIG * i)

        @pl.when(i + 2 < n_big)
        def _():
            start_loads(big0 + _BIG * (i + 2), _BIG, *big_in(slot))

        big_out(i).start()

        @pl.when(i < _N_FIRST)
        def _():
            copy(small(o_small, i), small(o_hbm, i), sem_so.at[_N_LAST]).start()

        j = (i >> 2) - last_load_quad

        @pl.when((j >= 0) & (j < _N_LAST) & ((i & 3) == 0))
        def _():
            head = last0 + _SMALL * j
            sem = sem_si.at[j]
            copy(k_hbm.at[pl.ds(head + 1, _SMALL - 1)],
                 k_small.at[pl.ds(_SMALL * j, _SMALL - 1)], sem).start()
            copy(k_hbm.at[jnp.minimum(head + _SMALL, n_heads - 1)],
                 k_small.at[_SMALL * j + _SMALL - 1], sem).start()
            copy(q_hbm.at[pl.ds(head, _SMALL)], small(q_small, j), sem).start()
            copy(v_hbm.at[pl.ds(head, _SMALL)], small(v_small, j), sem).start()

    jax.lax.fori_loop(0, n_big, big_step, None)

    def last_step(j, _):
        wait_loads(*small_in(j, j))
        run([small(x, j) for x in (q_small, k_small, v_small)]
            + [small(o_small, _N_FIRST + j)], last0 + _SMALL * j)
        last_out(j).start()

    jax.lax.fori_loop(0, _N_LAST, last_step, None)
    any_redo = jnp.max(jnp.max(redo_ref[...], axis=0)) > 0.0

    copy(o_small.at[pl.ds(0, big0)], o_hbm.at[pl.ds(0, big0)], sem_so.at[_N_LAST]).wait()
    big_out(n_big - 2).wait()
    big_out(n_big - 1).wait()
    for j in range(_N_LAST):
        last_out(j).wait()

    def redo_step(head, _):
        @pl.when(jnp.max(redo_ref[head]) > 0.0)
        def _():
            q, k, v, o = (x.at[0, 0] for x in (q_big, k_big, v_big, o_big))
            for src, dst in ((q_hbm, q), (k_hbm, k), (v_hbm, v)):
                copy(src.at[head], dst, sem_bi.at[0]).start()
            wait_loads((q, k, v), sem_bi.at[0])
            _head_exact(q, k, v, o, scale_log2e)
            out = copy(o, o_hbm.at[head], sem_bo.at[0])
            out.start()
            out.wait()

    @pl.when(any_redo)
    def _():
        jax.lax.fori_loop(0, n_heads, redo_step, None)


@jax.jit
def pallas_standalone__gqa_softmax__near_ridge_kernel(
    q: jax.Array,
    k: jax.Array,
    v: jax.Array,
):
    B, Hq, Sq, D = q.shape
    Hkv, Sk = k.shape[1], k.shape[2]
    assert Hq == Hkv and D == 192 and Sk == 512
    n = B * Hq
    qt = jnp.swapaxes(q, 2, 3).reshape(n, 3, D // 3, Sq)
    kt = jnp.swapaxes(k, 2, 3).reshape(n, D, Sk)
    vt = jnp.swapaxes(v, 2, 3).reshape(n, D, Sk)

    def buffers(heads_in, heads_out):
        return [pltpu.VMEM((*heads_in, 3, D // 3, Sq), q.dtype),
                pltpu.VMEM((*heads_in, D, Sk), k.dtype),
                pltpu.VMEM((*heads_in, D, Sk), v.dtype),
                pltpu.VMEM((*heads_out, D, Sq), q.dtype)]

    ot = pl.pallas_call(
        functools.partial(_attn_kernel, scale_log2e=(D ** -0.5) * _LOG2E),
        in_specs=[pl.BlockSpec(memory_space=pl.ANY)] * 3,
        out_specs=pl.BlockSpec(memory_space=pl.ANY),
        out_shape=jax.ShapeDtypeStruct((n, D, Sq), q.dtype),
        scratch_shapes=[
            *buffers((_SMALL * _N_FIRST,), (_SMALL * (_N_FIRST + _N_LAST),)),
            *buffers((2, _BIG), (2, _BIG)),
            pltpu.VMEM((3, 64, Sk // 2), _U32),
            pltpu.VMEM((3, Sk // 4, 128), _U32),
            pltpu.VMEM((1, 128), _F32),
            pltpu.VMEM((n, 8, 128), _F32),
            pltpu.SemaphoreType.DMA((_N_LAST,)),
            pltpu.SemaphoreType.DMA((_N_LAST + 1,)),
            pltpu.SemaphoreType.DMA((2,)),
            pltpu.SemaphoreType.DMA((2,)),
            *[pltpu.VMEM((1, Sk, 128), _F32)] * _S_SLOTS,
        ],
        compiler_params=pltpu.CompilerParams(
            vmem_limit_bytes=100 * 1024 * 1024,
            disable_bounds_checks=True,
            flags={"XLA_TPU_FORCE_LP_LLO_SCHEDULER": True},
        ),
    )(qt, kt, vt)
    return jnp.swapaxes(ot.reshape(B, Hq, D, Sq), 2, 3)
```
